```python
import os as _os
_os.environ.setdefault("JAX_PLATFORMS", "cpu")
import jax
import jax.numpy as jnp

def _softmax(x, axis=-1):
    return jax.nn.softmax(x, axis=axis)
def _gelu(x):
    return jax.nn.gelu(x, approximate=True)
def _silu(x):
    return jax.nn.silu(x)
def _sigmoid(x):
    return jax.nn.sigmoid(x)
def _layernorm(x, axis=-1, eps=1e-5):
    m = jnp.mean(x, axis=axis, keepdims=True)
    v = jnp.var(x, axis=axis, keepdims=True)
    return (x - m) / jnp.sqrt(v + eps)
def _scatter_add(tgt, idx, src, axis=0):
    return tgt.at[idx].add(src)
def _segment_sum(src, seg, n):
    return jax.ops.segment_sum(src, seg, n)
class _Rng:
    def __init__(self, key):
        self._k = key
    def _next(self):
        self._k, sub = jax.random.split(self._k)
        return sub
    def normal(self, shape):
        return jax.random.normal(self._next(), shape, dtype=jnp.bfloat16)
    def randint(self, lo, hi, shape):
        return jax.random.randint(self._next(), shape, lo, hi, dtype=jnp.int32)
    def uniform(self, shape, lo=0.0, hi=1.0):
        return jax.random.uniform(self._next(), shape, jnp.bfloat16, lo, hi)
    def permutation(self, n):
        return jax.random.permutation(self._next(), n)


kernel_name = 'gated_mix__softmax_full_mha__dense_activation_squared_relu__prompt'

def setup_inputs():
    _rng = _Rng(jax.random.key(int.from_bytes(__import__("os").urandom(4), "little")))
    _w = (lambda a: (lambda t: t.astype(jnp.bfloat16) if jnp.issubdtype(t.dtype, jnp.floating) else t)(jnp.asarray(a)))
    def _A_setup():
        B, S, D = 1, 2048, 640
        return {
            "x": _w((lambda *s: _rng.normal(s) * 0.05)(B, S, D)),
            "wqkv": _w((lambda *s: _rng.normal(s) * 0.4)(D, 3 * D)),
            "wo": _w((lambda *s: _rng.normal(s) * 0.05)(D, D)),
        }
    _A_in = _A_setup()

    def _B_setup():
        B, S, D, F = 1, 2048, 640, 1536
        return {
            "x": _w((lambda *s: _rng.normal(s) * 0.05)(B, S, D)),
            "w1": _w((lambda *s: _rng.normal(s) * 0.05)(D, F)),
            "b1": _w((lambda *s: _rng.normal(s) * 0.05)(F)),
            "w2": _w((lambda *s: _rng.normal(s) * 0.05)(F, D)),
            "b2": _w((lambda *s: _rng.normal(s) * 0.05)(D)),
        }
    _B_in = _B_setup()

    return {
        "A_x": _A_in["x"],
        "A_wqkv": _A_in["wqkv"],
        "A_wo": _A_in["wo"],
        "B_x": _B_in["x"],
        "B_w1": _B_in["w1"],
        "B_b1": _B_in["b1"],
        "B_w2": _B_in["w2"],
        "B_b2": _B_in["b2"],
        "gate_w": _w((lambda *s: _rng.normal(s) * 0.05)(640) * 16.0),
    }

def reference(A_x, A_wqkv, A_wo, B_x, B_w1, B_b1, B_w2, B_b2, gate_w):
    def _A_ref(x, wqkv, wo):
        B, S, D = x.shape
        H = 32; Dh = D // H
        qkv = (lambda x, *d: x.transpose(*d))((x @ wqkv).reshape(B, S, 3, H, Dh), 2, 0, 3, 1, 4)
        q, k, v = qkv[0], qkv[1], qkv[2]
        scale = Dh ** -0.5
        scores = jnp.einsum("bhqd,bhkd->bhqk", q, k) * scale
        p = _softmax(scores, axis=-1)
        o = jnp.einsum("bhqk,bhkd->bhqd", p, v)
        return (lambda x, *d: x.transpose(*d))(o, 0, 2, 1, 3).reshape(B, S, D) @ wo

    def _B_ref(x, w1, b1, w2, b2):
        h = jnp.einsum("bsd,df->bsf", x, w1) + b1
        zero = jnp.zeros_like(h)
        r = jnp.where(h > zero, h, zero)
        h = r * r
        out = jnp.einsum("bsf,fd->bsd", h, w2) + b2
        return out

    x = A_x
    g = _sigmoid((x * gate_w).sum(-1, keepdims=True))
    a = _A_ref(x, A_wqkv, A_wo)
    b = _B_ref(x, B_w1, B_b1, B_w2, B_b2)
    return g * a + (1 - g) * b
```

```python
import functools
import math
import jax
import jax.numpy as jnp
import jax.experimental.pallas as pl
import jax.experimental.pallas.tpu as pltpu

S = 2048
D = 640
H = 32
DH = 20
F = 1536
LANE = 128
VROWS = 24
NKB = D // LANE

STRADDLE = [h for h in range(H) if (DH * h) // LANE != (DH * h + DH - 1) // LANE]


def make_kernel(TQ, CK, RC, HPB):
    NQ = S // TQ
    NC = S // CK
    NR = S // RC
    NB = H // HPB
    qscale = (DH ** -0.5) * math.log2(math.e)

    def kidx_of(h):
        lo = (DH * h) // LANE
        hi = (DH * h + DH - 1) // LANE
        return jnp.where(lo == hi, lo, NKB + lo)

    def kernel(x_hbm, wqkv_hbm, wo_hbm, w1_hbm, b1_ref, w2_hbm, b2_ref, gw_ref, o_ref,
               x_ref, wqkv_ref, wo_ref, w1_ref, w2_ref, sems,
               kb_ref, qm_ref, vt_ref, s_ref, m_ref, ot_ref, otc_ref):
        step = pl.program_id(0)

        def x_copy(r):
            return pltpu.make_async_copy(x_hbm.at[pl.ds(r * RC, RC), :], x_ref.at[pl.ds(r * RC, RC), :], sems.at[r])

        def w_copy(p):
            return pltpu.make_async_copy(wqkv_hbm.at[:, pl.ds(p * D, D)], wqkv_ref.at[p], sems.at[NR + p])

        late = [pltpu.make_async_copy(wo_hbm, wo_ref, sems.at[NR + 3]),
                pltpu.make_async_copy(w1_hbm, w1_ref, sems.at[NR + 4]),
                pltpu.make_async_copy(w2_hbm, w2_ref, sems.at[NR + 5])]

        def qk_chunk(t, h, c, kidx):
            return jnp.dot(kb_ref[kidx, pl.ds(c * CK, CK), :], qm_ref[t * H + h],
                           preferred_element_type=jnp.float32)

        def colmax8(s):
            return jnp.max(s.reshape(CK // 8, 8, TQ), axis=0)

        @pl.when(step == 0)
        def _prologue():
            x_copy(0).start()
            w_copy(0).start()
            for r in range(1, NR):
                x_copy(r).start()
            w_copy(1).start()
            w_copy(2).start()
            for cp in late:
                cp.start()

            lane = jax.lax.broadcasted_iota(jnp.int32, (RC, LANE), 1)
            row = jax.lax.broadcasted_iota(jnp.int32, (LANE, RC), 0)
            vrow = jax.lax.broadcasted_iota(jnp.int32, (8, RC), 0)

            def q_rows(r, _):
                r0 = pl.multiple_of(r * RC, RC)
                x_copy(r).wait()
                xc = x_ref[pl.ds(r0, RC), :]
                q = jnp.dot(xc, wqkv_ref[0], preferred_element_type=jnp.float32) * qscale
                qt = q.T
                for h in range(H):
                    b = (DH * h) // LANE
                    t0 = DH * h - b * LANE
                    blk = qt[b * LANE:(b + 1) * LANE, :]
                    if h in STRADDLE:
                        blk2 = qt[(b + 1) * LANE:(b + 2) * LANE, :]
                        w = jnp.where(row >= t0, blk, jnp.where(row < t0 + DH - LANE, blk2, 0.0))
                    else:
                        w = jnp.where((row >= t0) & (row < t0 + DH), blk, 0.0)
                    w = w.astype(jnp.bfloat16)
                    if RC == TQ:
                        qm_ref[r * H + h] = w
                    else:
                        per = TQ // RC
                        qm_ref[(r // per) * H + h, :, pl.ds(pl.multiple_of((r % per) * RC, RC), RC)] = w
                return 0

            def kv_rows(r, _):
                r0 = pl.multiple_of(r * RC, RC)
                xc = x_ref[pl.ds(r0, RC), :]
                v = jnp.dot(xc, wqkv_ref[2], preferred_element_type=jnp.float32)
                vt = v.T
                for h in range(H):
                    vt_ref[h, 0:16, pl.ds(r0, RC)] = vt[DH * h:DH * h + 16, :]
                    lo = DH * h + 16
                    if lo + 8 <= D:
                        tail = vt[lo:lo + 8, :]
                    else:
                        tail = jnp.concatenate([vt[lo:lo + 4, :], vt[lo:lo + 4, :]], axis=0)
                    tail = jnp.where(vrow < 4, tail, jnp.where(vrow == 4, 1.0, 0.0))
                    vt_ref[h, 16:24, pl.ds(r0, RC)] = tail
                k = jnp.dot(xc, wqkv_ref[1], preferred_element_type=jnp.float32)
                for b in range(NKB):
                    kb_ref[b, pl.ds(r0, RC), :] = k[:, b * LANE:(b + 1) * LANE].astype(jnp.bfloat16)
                for h in STRADDLE:
                    b = (DH * h) // LANE
                    t0 = DH * h - b * LANE
                    mrg = jnp.where(lane >= t0, k[:, b * LANE:(b + 1) * LANE], k[:, (b + 1) * LANE:(b + 2) * LANE])
                    kb_ref[NKB + b, pl.ds(r0, RC), :] = mrg.astype(jnp.bfloat16)
                return 0

            w_copy(0).wait()
            jax.lax.fori_loop(0, NR, q_rows, 0)
            w_copy(1).wait()
            w_copy(2).wait()
            jax.lax.fori_loop(0, NR, kv_rows, 0)
            for i in range(HPB):
                m = None
                for c in range(NC):
                    s = qk_chunk(0, i, c, kidx_of(i))
                    s_ref[i, pl.ds(c * CK, CK), :] = s
                    cm = colmax8(s)
                    m = cm if m is None else jnp.maximum(m, cm)
                m_ref[i] = m

        def stage(i, h, tn, hn, m8):
            kidx = kidx_of(hn)
            m = jnp.max(m8, axis=0, keepdims=True)
            m_new = None
            acc = None
            for c in range(NC):
                p = jnp.exp2(s_ref[i, pl.ds(c * CK, CK), :] - m)
                s = qk_chunk(tn, hn, c, kidx)
                s_ref[i, pl.ds(c * CK, CK), :] = s
                cm = colmax8(s)
                m_new = cm if m_new is None else jnp.maximum(m_new, cm)
                pv = jnp.dot(vt_ref[h, :, pl.ds(c * CK, CK)], p, preferred_element_type=jnp.float32)
                acc = pv if acc is None else acc + pv
            inv = 1.0 / acc[DH:DH + 1, :]
            ot_ref[h] = acc * inv
            return m_new

        def block(j, ms):
            last = j == (NB - 1)
            tn = jnp.where(last, jnp.minimum(step + 1, NQ - 1), step)
            hb = jnp.where(last, 0, (j + 1) * HPB)
            return tuple(stage(i, j * HPB + i, tn, hb + i, ms[i]) for i in range(HPB))

        ms = jax.lax.fori_loop(0, NB, block, tuple(m_ref[i] for i in range(HPB)))
        for i in range(HPB):
            m_ref[i] = ms[i]

        @pl.when(step == 0)
        def _():
            for cp in late:
                cp.wait()

        for h in range(H):
            otc_ref[DH * h:DH * h + DH, :] = ot_ref[h, 0:DH, :]
        o = otc_ref[...].T.astype(jnp.bfloat16)
        a = jnp.dot(o, wo_ref[...], preferred_element_type=jnp.float32)
        r0 = pl.multiple_of(step * TQ, TQ)
        xt = x_ref[pl.ds(r0, TQ), :]
        hid = jnp.dot(xt, w1_ref[...], preferred_element_type=jnp.float32) + b1_ref[...].astype(jnp.float32)[None, :]
        hid = jnp.maximum(hid, 0.0)
        hid = (hid * hid).astype(jnp.bfloat16)
        bb = jnp.dot(hid, w2_ref[...], preferred_element_type=jnp.float32) + b2_ref[...].astype(jnp.float32)[None, :]
        gl = jnp.sum(xt.astype(jnp.float32) * gw_ref[...].astype(jnp.float32)[None, :], axis=-1, keepdims=True)
        g = jax.nn.sigmoid(gl)
        o_ref[...] = (g * a + (1.0 - g) * bb).astype(o_ref.dtype)

    return kernel


def build(TQ=512, CK=256, RC=512, HPB=2):
    NQ = S // TQ
    NR = S // RC

    def fn(A_x, A_wqkv, A_wo, B_x, B_w1, B_b1, B_w2, B_b2, gate_w):
        x = A_x.reshape(S, D)
        full = lambda shape: pl.BlockSpec(shape, lambda i: (0,) * len(shape))
        hbm = pl.BlockSpec(memory_space=pl.ANY)
        out = pl.pallas_call(
            make_kernel(TQ, CK, RC, HPB),
            grid=(NQ,),
            in_specs=[hbm, hbm, hbm, hbm, full((F,)), hbm, full((D,)), full((D,))],
            out_specs=pl.BlockSpec((TQ, D), lambda i: (i, 0)),
            out_shape=jax.ShapeDtypeStruct((S, D), jnp.bfloat16),
            scratch_shapes=[
                pltpu.VMEM((S, D), jnp.bfloat16),
                pltpu.VMEM((3, D, D), jnp.bfloat16),
                pltpu.VMEM((D, D), jnp.bfloat16),
                pltpu.VMEM((D, F), jnp.bfloat16),
                pltpu.VMEM((F, D), jnp.bfloat16),
                pltpu.SemaphoreType.DMA((NR + 6,)),
                pltpu.VMEM((NKB + len(STRADDLE), S, LANE), jnp.bfloat16),
                pltpu.VMEM((NQ * H, LANE, TQ), jnp.bfloat16),
                pltpu.VMEM((H, VROWS, S), jnp.float32),
                pltpu.VMEM((HPB, S, TQ), jnp.float32),
                pltpu.VMEM((HPB, 8, TQ), jnp.float32),
                pltpu.VMEM((H, VROWS, TQ), jnp.float32),
                pltpu.VMEM((D, TQ), jnp.float32),
            ],
            compiler_params=pltpu.CompilerParams(
                dimension_semantics=("arbitrary",),
                vmem_limit_bytes=100 * 1024 * 1024),
        )(x, A_wqkv, A_wo, B_w1, B_b1, B_w2, B_b2, gate_w)
        return out.reshape(1, S, D)
    return fn


@jax.jit
def pallas_gated_mix__softmax_full_mha__dense_activation_squared_relu__prompt_kernel(
    A_x: jax.Array,
    A_wqkv: jax.Array,
    A_wo: jax.Array,
    B_x: jax.Array,
    B_w1: jax.Array,
    B_b1: jax.Array,
    B_w2: jax.Array,
    B_b2: jax.Array,
    gate_w: jax.Array,
):
    return build()(A_x, A_wqkv, A_wo, B_x, B_w1, B_b1, B_w2, B_b2, gate_w)
```

```python
import math
import jax
import jax.numpy as jnp
import jax.experimental.pallas as pl
import jax.experimental.pallas.tpu as pltpu

S = 2048
D = 640
H = 32
DH = 20
F = 1536
LANE = 128
VROWS = 24
NKB = D // LANE
f32 = jnp.float32
bf16 = jnp.bfloat16

STRADDLE = [h for h in range(H) if (DH * h) // LANE != (DH * h + DH - 1) // LANE]

POS12 = (0.04, 0.08, 0.12, 0.2, 0.35, 0.55, 0.65, 0.75, 0.85, 0.92, 1.0, 1.0)


def make_kernel(TQ, CK, RC, TE, RVS, POSL, OPQ, NP):
    NG = S // TQ
    NC = S // CK
    NU = NG * NC
    NR = S // RC
    NJ = TQ // LANE
    G8 = CK // 8
    rv = [RVS[c % len(RVS)] // 8 for c in range(NC)]
    cstart = [sum(G8 - rv[cc] for cc in range(c)) for c in range(NC + 1)]
    vstart = [sum(rv[:c]) for c in range(NC + 1)]
    NV = vstart[NC]
    PPU = -(-(NV * NJ) // NC)
    CPR = RC // CK
    assert CPR % len(RVS) == 0
    qscale = (DH ** -0.5) * math.log2(math.e)

    def kidx_of(h):
        if isinstance(h, int):
            lo, hi = (DH * h) // LANE, (DH * h + DH - 1) // LANE
            return lo if lo == hi else NKB + lo
        lo = (DH * h) // LANE
        hi = (DH * h + DH - 1) // LANE
        return jnp.where(lo == hi, lo, NKB + lo)

    def kernel(x_hbm, wqkv_hbm, wo_hbm, w1_hbm, b1_ref, w2_hbm, b2_ref, gw_ref, o_ref,
               x_ref, wqkv_ref, wo_ref, w1_ref, w2_ref, sems,
               kb_ref, qm_ref, vt_ref, s_ref, ot_ref, otc_ref, bb_ref, ko_ref, qt_ref, kbc_ref, hid_ref, z_ref):
        step = pl.program_id(0)

        def x_copy(r):
            return pltpu.make_async_copy(x_hbm.at[pl.ds(r * RC, RC), :], x_ref.at[pl.ds(r * RC, RC), :], sems.at[r])

        def w_copy(p):
            return pltpu.make_async_copy(wqkv_hbm.at[:, pl.ds(p * D, D)], wqkv_ref.at[p], sems.at[NR + p])

        late = [pltpu.make_async_copy(wo_hbm, wo_ref, sems.at[NR + 3]),
                pltpu.make_async_copy(w1_hbm, w1_ref, sems.at[NR + 4]),
                pltpu.make_async_copy(w2_hbm, w2_ref, sems.at[NR + 5])]

        def make_kbc(h, i):
            ko = ko_ref[h, pl.ds(i * 8, 8), :]
            for d in range(DH):
                kbc_ref[d, pl.ds(i * 8, 8), :] = jnp.broadcast_to(ko[:, d:d + 1], (8, LANE))

        def block(h, hn, ms, extra=None):
            mnxt = [None] * NG
            P = {}
            if hn is not None:
                kidx = kidx_of(hn)
                hn2 = min(hn + 1, H - 1) if isinstance(hn, int) else jnp.minimum(hn + 1, H - 1)

            def ensure_p(g, rg):
                if h is not None and (g, rg) not in P:
                    P[(g, rg)] = jnp.exp2(s_ref[g, pl.ds(rg * 8, 8), :] - ms[g])

            def vpu_piece(cm, g, c, r, j):
                rg = c * G8 + r
                i = vstart[c] + r
                ensure_p(g, rg)
                hz = hn + z_ref[i % 4] if OPQ else hn
                acc = None
                for d in range(DH):
                    t = kbc_ref[d, pl.ds(i * 8, 8), :] * qt_ref[hz, pl.ds(d, 1), pl.ds(g * TQ + j * LANE, LANE)]
                    acc = t if acc is None else acc + t
                s_ref[g, pl.ds(rg * 8, 8), pl.ds(j * LANE, LANE)] = acc
                cm[j] = jnp.maximum(cm[j], acc)
                if g == NG - 1 and j == NJ - 1:
                    make_kbc(hn2, i)

            acc = None
            for u in range(NU):
                g, c = divmod(u, NC)
                if hn is not None:
                    if c == 0:
                        cm = [None] * NJ
                        queue = []
                    queue += [(g, c, r, j) for r in range(rv[c]) for j in range(NJ)]
                    n = len(queue) if c == NC - 1 else min(PPU, len(queue))
                    mine, queue = queue[:n], queue[n:]
                    L = G8 - rv[c]
                    if len(mine) == len(POSL):
                        pos = [max(0, int(round(POSL[k] * L)) - 1) for k in range(len(mine))]
                    else:
                        pos = [int(round((k + 1) / len(mine) * L)) - 1 for k in range(len(mine))]
                    for r in range(rv[c], G8):
                        ensure_p(g, c * G8 + r)
                    kk = pltpu.bitcast(kb_ref[kidx, pl.ds(cstart[c] * 4, L * 4), :], bf16)
                    qq = pltpu.bitcast(qm_ref[hn, :, pl.ds(g * TQ, TQ)], bf16)
                    sn = jnp.dot(kk, qq, preferred_element_type=f32)
                    loc = None
                    for i in range(L):
                        part = sn[i * 8:(i + 1) * 8, :]
                        s_ref[g, pl.ds((c * G8 + rv[c] + i) * 8, 8), :] = part
                        loc = part if loc is None else jnp.maximum(loc, part)
                        if i == L - 1 or i in pos:
                            for j in range(NJ):
                                lj = loc[:, j * LANE:(j + 1) * LANE]
                                cm[j] = lj if cm[j] is None else jnp.maximum(cm[j], lj)
                            loc = None
                        for k in range(len(mine)):
                            if pos[k] == i:
                                vpu_piece(cm, *mine[k])
                    if c == NC - 1:
                        m = jnp.concatenate(cm, axis=1)
                        mnxt[g] = jnp.broadcast_to(jnp.max(m, axis=0, keepdims=True), (8, TQ))
                if h is not None:
                    for rg in range(c * G8, (c + 1) * G8):
                        ensure_p(g, rg)
                    p = jnp.concatenate([P[(g, rg)] for rg in range(c * G8, (c + 1) * G8)], axis=0)
                    pv = jnp.dot(vt_ref[h, :, pl.ds(c * CK, CK)], p, preferred_element_type=f32)
                    acc = pv if c == 0 else pv + acc
                    if c == NC - 1:
                        inv = 1.0 / acc[DH:DH + 1, :]
                        ot_ref[h, :, pl.ds(g * TQ, TQ)] = acc * inv
                if extra is not None:
                    extra(u)
            return tuple(mnxt)

        def ffn_part(t, i, n):
            r0 = pl.multiple_of(t * TE, TE)
            half = n // 2
            if i < half:
                w = F // half
                xt = x_ref[pl.ds(r0, TE), :]
                hid = jnp.dot(xt, w1_ref[:, i * w:(i + 1) * w], preferred_element_type=f32)
                hid = hid + b1_ref[pl.ds(i * w, w)].astype(f32)[None, :]
                hid = jnp.maximum(hid, 0.0)
                hid_ref[:, i * w:(i + 1) * w] = (hid * hid).astype(bf16)
            else:
                i -= half
                w = TE // half
                bb_ref[i * w:(i + 1) * w, :] = (
                    jnp.dot(hid_ref[i * w:(i + 1) * w, :], w2_ref[...], preferred_element_type=f32)
                    + b2_ref[...].astype(f32)[None, :])

        @pl.when(step == 0)
        def _attention():
            x_copy(0).start()
            w_copy(0).start()
            for r in range(1, NR):
                x_copy(r).start()
            w_copy(1).start()
            w_copy(2).start()
            for cp in late:
                cp.start()
            for i in range(4):
                z_ref[i] = 0

            def zero(h, _):
                qm_ref[h] = jnp.zeros((LANE // 2, S), jnp.uint32)
                return 0
            jax.lax.fori_loop(0, H, zero, 0)

            lane = jax.lax.broadcasted_iota(jnp.int32, (RC, LANE), 1)
            row16 = jax.lax.broadcasted_iota(jnp.int32, (16, RC), 0)
            vrow = jax.lax.broadcasted_iota(jnp.int32, (8, RC), 0)

            def head_rows(t, h, fill):
                lo = DH * h + 16
                if lo + 8 <= D:
                    tail = t[lo:lo + 8, :]
                else:
                    tail = jnp.concatenate([t[lo:lo + 4, :], t[lo:lo + 4, :]], axis=0)
                return t[DH * h:DH * h + 16, :], jnp.where(vrow < 4, tail, fill)

            def q_rows(r, _):
                r0 = pl.multiple_of(r * RC, RC)
                x_copy(r).wait()
                xc = x_ref[pl.ds(r0, RC), :]
                q = jnp.dot(xc, wqkv_ref[0], preferred_element_type=f32) * qscale
                qt = q.T
                for h in range(H):
                    lo, hi = DH * h, DH * h + DH
                    for a in range(lo // 16 * 16, hi, 16):
                        blk = qt[a:a + 16, :]
                        if a < lo:
                            blk = jnp.where(row16 >= lo - a, blk, 0.0)
                        if a + 16 > hi:
                            blk = jnp.where(row16 < hi - a, blk, 0.0)
                        qm_ref[h, pl.ds(a % LANE // 2, 8), pl.ds(r0, RC)] = pltpu.bitcast(blk.astype(bf16), jnp.uint32)
                if NV:
                    qr = qt.astype(bf16).astype(f32)
                    for h in range(H):
                        top, tail = head_rows(qr, h, 0.0)
                        qt_ref[h, 0:16, pl.ds(r0, RC)] = top
                        qt_ref[h, 16:24, pl.ds(r0, RC)] = tail
                return 0

            MR = cstart[CPR] * 4
            VR = vstart[CPR] * 8

            def kv_rows(r, _):
                r0 = pl.multiple_of(r * RC, RC)
                xc = x_ref[pl.ds(r0, RC), :]
                v = jnp.dot(xc, wqkv_ref[2], preferred_element_type=f32)
                vt = v.T
                fill = jnp.where(vrow == 4, 1.0, 0.0)
                for h in range(H):
                    top, tail = head_rows(vt, h, fill)
                    vt_ref[h, 0:16, pl.ds(r0, RC)] = top
                    vt_ref[h, 16:24, pl.ds(r0, RC)] = tail
                k = jnp.dot(xc, wqkv_ref[1], preferred_element_type=f32)
                blks = [k[:, b * LANE:(b + 1) * LANE] for b in range(NKB)]
                for h in STRADDLE:
                    b = (DH * h) // LANE
                    blks.append(jnp.where(lane >= DH * h - b * LANE, blks[b], blks[b + 1]))
                for b in range(len(blks)):
                    for cc in range(CPR):
                        src = blks[b][cc * CK + rv[cc] * 8:(cc + 1) * CK, :].astype(bf16)
                        dst = pl.multiple_of(r * MR + cstart[cc] * 4, 8)
                        kb_ref[b, pl.ds(dst, (G8 - rv[cc]) * 4), :] = pltpu.bitcast(src, jnp.uint32)
                for cc in range(CPR):
                    if rv[cc] == 0:
                        continue
                    for h in range(H):
                        b = (DH * h) // LANE
                        t0 = DH * h - b * LANE
                        src = blks[NKB + b if h in STRADDLE else b][cc * CK:cc * CK + rv[cc] * 8, :]
                        src = src.astype(bf16).astype(f32)
                        if t0:
                            src = pltpu.roll(src, LANE - t0, 1)
                        dst = pl.multiple_of(r * VR + vstart[cc] * 8, 8)
                        ko_ref[h, pl.ds(dst, rv[cc] * 8), :] = src
                return 0

            w_copy(0).wait()
            jax.lax.fori_loop(0, NR, q_rows, 0)
            w_copy(1).wait()
            w_copy(2).wait()
            jax.lax.fori_loop(0, NR, kv_rows, 0)

            for i in range(NV):
                make_kbc(0, i)
            ms = block(None, 0, None)
            ms = jax.lax.fori_loop(0, H - 1, lambda h, ms: block(h, h + 1, ms), ms)
            for cp in late:
                cp.wait()

            def extra(u):
                every = NU // NP
                if u % every == 0:
                    ffn_part(0, u // every, NP)
            block(H - 1, None, ms, extra=extra)

        @pl.when(step > 0)
        def _():
            for i in range(2):
                ffn_part(step, i, 2)

        r0 = pl.multiple_of(step * TE, TE)
        for h in range(H):
            otc_ref[DH * h:DH * h + DH, :] = ot_ref[h, 0:DH, pl.ds(r0, TE)]
        o = otc_ref[...].T.astype(bf16)
        a = jnp.dot(o, wo_ref[...], preferred_element_type=f32)
        xt = x_ref[pl.ds(r0, TE), :]
        gl = jnp.sum(xt.astype(f32) * gw_ref[...].astype(f32)[None, :], axis=-1, keepdims=True)
        g = jax.nn.sigmoid(gl)
        o_ref[...] = (g * a + (1.0 - g) * bb_ref[...]).astype(o_ref.dtype)

    scratch = [
        pltpu.VMEM((S, D), bf16),
        pltpu.VMEM((3, D, D), bf16),
        pltpu.VMEM((D, D), bf16),
        pltpu.VMEM((D, F), bf16),
        pltpu.VMEM((F, D), bf16),
        pltpu.SemaphoreType.DMA((NR + 6,)),
        pltpu.VMEM((NKB + len(STRADDLE), cstart[NC] * 4, LANE), jnp.uint32),
        pltpu.VMEM((H, LANE // 2, S), jnp.uint32),
        pltpu.VMEM((H, VROWS, S), f32),
        pltpu.VMEM((NG, S, TQ), f32),
        pltpu.VMEM((H, VROWS, S), f32),
        pltpu.VMEM((D, TE), f32),
        pltpu.VMEM((TE, D), f32),
        pltpu.VMEM((H, max(NV, 1) * 8, LANE), f32),
        pltpu.VMEM((H, VROWS, S), f32),
        pltpu.VMEM((DH, max(NV, 1) * 8, LANE), f32),
        pltpu.VMEM((TE, F), bf16),
        pltpu.SMEM((4,), jnp.int32),
    ]
    return kernel, scratch


def build(TQ=512, CK=256, RC=512, TE=512, RVS=(32, 16), POSL=POS12, OPQ=1, NP=8):
    kernel, scratch = make_kernel(TQ, CK, RC, TE, RVS, POSL, OPQ, NP)

    def fn(A_x, A_wqkv, A_wo, B_x, B_w1, B_b1, B_w2, B_b2, gate_w):
        x = A_x.reshape(S, D)
        full = lambda shape: pl.BlockSpec(shape, lambda i: (0,) * len(shape))
        hbm = pl.BlockSpec(memory_space=pl.ANY)
        out = pl.pallas_call(
            kernel,
            grid=(S // TE,),
            in_specs=[hbm, hbm, hbm, hbm, full((F,)), hbm, full((D,)), full((D,))],
            out_specs=pl.BlockSpec((TE, D), lambda i: (i, 0)),
            out_shape=jax.ShapeDtypeStruct((S, D), bf16),
            scratch_shapes=scratch,
            compiler_params=pltpu.CompilerParams(
                dimension_semantics=("arbitrary",),
                vmem_limit_bytes=110 * 1024 * 1024),
        )(x, A_wqkv, A_wo, B_w1, B_b1, B_w2, B_b2, gate_w)
        return out.reshape(1, S, D)
    return fn


@jax.jit
def pallas_gated_mix__softmax_full_mha__dense_activation_squared_relu__prompt_kernel(
    A_x: jax.Array,
    A_wqkv: jax.Array,
    A_wo: jax.Array,
    B_x: jax.Array,
    B_w1: jax.Array,
    B_b1: jax.Array,
    B_w2: jax.Array,
    B_b2: jax.Array,
    gate_w: jax.Array,
):
    return build()(A_x, A_wqkv, A_wo, B_x, B_w1, B_b1, B_w2, B_b2, gate_w)
```

```python
import math
import jax
import jax.numpy as jnp
import jax.experimental.pallas as pl
import jax.experimental.pallas.tpu as pltpu

S = 2048
D = 640
H = 32
DH = 20
F = 1536
LANE = 128
VROWS = 24
KD = 32
FB = S // H
NKT = D // LANE
f32 = jnp.float32
bf16 = jnp.bfloat16
u32 = jnp.uint32


def _ds(i, n):
    return pl.ds(i * n, n) if isinstance(i, int) else pl.ds(pl.multiple_of(i * n, n), n)


def make_kernel(TQ, CK, RC, RVG, POFF, FR, FSKIP, ONLY, PRO, ORDER, PAD, XW, PREPC):
    NG = S // TQ
    NC = S // CK
    NU = NG * NC
    NR = S // RC
    NJ = TQ // LANE
    G8 = CK // 8
    rvg = [[int(ch) for ch in pat] for pat in RVG]
    rv = [max(rvg[g][c] for g in range(NG)) for c in range(NC)]
    last_use = {(c, r): max(g for g in range(NG) if rvg[g][c] > r) for c in range(NC) for r in range(rv[c])}
    vstart = [sum(rv[:c]) for c in range(NC + 1)]
    NV = vstart[NC]
    RMAX = max(max(rv), 2)
    qscale = (DH ** -0.5) * math.log2(math.e)
    fdots = [(ph, rp, th, sub) for ph in range(2) for rp in range(FB // FR) for th in range(3) for sub in range(5)]
    funits = [u for u in range(NU) if u not in FSKIP]
    fmap = {}
    for k, fd in enumerate(fdots):
        fmap.setdefault(funits[k * len(funits) // len(fdots)], []).append(fd)

    def kernel(x_hbm, wqkv_hbm, wo_hbm, w1_hbm, b1_hbm, w2_hbm, b2_hbm, gw_hbm, o_hbm,
               x_ref, wqkv_ref, wo_ref, w1_ref, w2_ref, sems,
               kb_ref, qm_ref, vt_ref, s_ref, ot_ref, otc_ref, bb_ref, qt_ref, kbc_ref, hid_ref, z_ref, ko_ref,
               w1p_ref, w2p_ref, wop_ref, bf_ref, o_ref, osems, m_ref, gb_ref, inv_ref, op_ref, xp_ref,
               b1_ref, b2_ref, gw_ref):

        def x_copy(r):
            return pltpu.make_async_copy(x_hbm.at[pl.ds(r * RC, RC), :], x_ref.at[pl.ds(r * RC, RC), :], sems.at[r])

        def w_copy(p):
            return pltpu.make_async_copy(wqkv_hbm.at[:, pl.ds(p * D, D)], wqkv_ref.at[p], sems.at[NR + p])

        late = [pltpu.make_async_copy(w1_hbm, w1_ref, sems.at[NR + 3]),
                pltpu.make_async_copy(w2_hbm, w2_ref, sems.at[NR + 4]),
                pltpu.make_async_copy(wo_hbm, wo_ref, sems.at[NR + 5]),
                pltpu.make_async_copy(b1_hbm, b1_ref, sems.at[NR + 6]),
                pltpu.make_async_copy(b2_hbm, b2_ref, sems.at[NR + 7])]

        def o_copy(g):
            return pltpu.make_async_copy(o_ref.at[_ds(g, TQ), :], o_hbm.at[_ds(g, TQ), :], osems.at[g])

        def colmax8(s):
            return jnp.max(s.reshape(s.shape[0] // 8, 8, s.shape[1]), axis=0) if s.shape[0] > 8 else s

        def after(x, link):
            lk = link if x.dtype == f32 else pltpu.bitcast(link, x.dtype)
            lk = jnp.concatenate([lk] * (x.shape[1] // LANE), axis=1)
            lk = jnp.concatenate([lk] * (x.shape[0] // 8), axis=0)
            return jnp.where(jnp.full(x.shape, z_ref[0]) != 0, lk, x)

        def make_kbc(h, c, r, link=None):
            ko = ko_ref[h, pl.ds((c * RMAX + r) * 8, 8), :]
            if link is not None:
                ko = after(ko, link)
            for d in range(DH):
                kbc_ref[vstart[c] + r, d] = jnp.broadcast_to(ko[:, d:d + 1], (8, LANE))

        def ffn_dot(fb, st, ph, rp, th, sub, FR=FR):
            r0 = fb * FB + rp * FR
            if not isinstance(r0, int):
                r0 = pl.multiple_of(r0, FR)
            hcols = slice(th * 512, (th + 1) * 512)
            hrows = slice(rp * FR // 2, (rp + 1) * FR // 2)
            if ph == 0:
                xt = pltpu.bitcast(xp_ref[fb, rp * FR // 2:(rp + 1) * FR // 2, sub * LANE:(sub + 1) * LANE], bf16)
                w = pltpu.bitcast(w1p_ref[sub * 64:(sub + 1) * 64, hcols], bf16)
                o = jnp.dot(xt, w, preferred_element_type=f32)
                st["a"] = o + (bf_ref[0:1, hcols] if sub == 0 else st["a"])
                if sub == 4:
                    hid = jnp.maximum(st["a"], 0.0)
                    hid_ref[hrows, hcols] = pltpu.bitcast((hid * hid).astype(bf16), u32)
            else:
                hd = pltpu.bitcast(hid_ref[hrows, hcols], bf16)
                w = pltpu.bitcast(w2p_ref[th * 256:(th + 1) * 256, sub * LANE:(sub + 1) * LANE], bf16)
                o = jnp.dot(hd, w, preferred_element_type=f32)
                dst = (pl.ds(r0, FR), pl.ds(sub * LANE, LANE))
                bb_ref[dst] = o if th == 0 else o + bb_ref[dst]

        def block(h, hn, ms, extra=None, rvg=rvg):
            mnxt = [None] * NG
            fst = {}
            hn2 = min(hn + 1, H - 1) if isinstance(hn, int) else jnp.minimum(hn + 1, H - 1)

            def vpu_piece(g, c, r, j):
                i = vstart[c] + r

                def term(d):
                    return kbc_ref[i, d] * qt_ref[hn, pl.ds(d, 1), pl.ds(g * TQ + j * LANE, LANE)]
                acc = jax.lax.fori_loop(1, DH, lambda d, a: a + term(d), term(0), unroll=True)
                s_ref[g, pl.ds((c * G8 + r) * 8, 8), pl.ds(j * LANE, LANE)] = acc
                if g == last_use[(c, r)] and j == NJ - 1:
                    make_kbc(hn2, c, r)
                return acc

            acc = None
            for u in range(NU):
                g, c = divmod(u, NC)
                if h is not None:
                    s = s_ref[g, pl.ds(c * CK, CK), :].reshape(G8, 8, TQ)
                    p = jnp.exp2(s - ms[g][None]).reshape(CK, TQ)
                if c == 0:
                    cm = [None] * NJ
                    queue = []
                    taken = 0
                    rv = rvg[g]
                queue += [(g, c, r, j) for r in range(rv[c]) for j in range(NJ)]
                n = len(queue) if c == NC - 1 else min(int(round(sum(rv) * NJ * (c + 1) / NC)) - taken, len(queue))
                taken += n
                mine, queue = queue[:n], queue[n:]
                L = G8 - rv[c]
                pos = [max(1, int(round((k + 1) / len(mine) * (L + POFF) - POFF))) for k in range(len(mine))]
                kk = pltpu.bitcast(kb_ref[hn, pl.ds((c * G8 + rv[c]) * 4, L * 4), :], bf16)[:, 0:KD]
                qq = pltpu.bitcast(qm_ref[hn, :, pl.ds(g * TQ, TQ)], bf16)
                sn = jnp.dot(kk, qq, preferred_element_type=f32)
                s_ref[g, pl.ds((c * G8 + rv[c]) * 8, L * 8), :] = sn
                done = 0
                for k in range(len(mine) + 1):
                    upto = pos[k] if k < len(mine) else L
                    if upto > done:
                        lj = colmax8(sn[done * 8:upto * 8, :])
                        for j in range(NJ):
                            x = lj[:, j * LANE:(j + 1) * LANE]
                            cm[j] = x if cm[j] is None else jnp.maximum(cm[j], x)
                        done = upto
                    if k < len(mine):
                        j = mine[k][3]
                        cm[j] = jnp.maximum(cm[j], vpu_piece(*mine[k]))
                if c == NC - 1:
                    m = jnp.concatenate(cm, axis=1)
                    mnxt[g] = jnp.broadcast_to(jnp.max(m, axis=0, keepdims=True), (8, TQ))
                if h is not None:
                    pv = jnp.dot(vt_ref[h, :, pl.ds(c * CK, CK)], p, preferred_element_type=f32)
                    acc = pv if c == 0 else pv + acc
                    if c == NC - 1:
                        for j in range(NJ):
                            ot_ref[g * NJ + j, _ds(h, VROWS), :] = acc[:, j * LANE:(j + 1) * LANE]
                    for fd in fmap.get(u, []):
                        ffn_dot(h, fst, *fd)
                if extra is not None:
                    extra(u, sn[0:8, 0:LANE])
            return tuple(mnxt)

        if ONLY:
            ms = tuple(s_ref[g, 0:8, :] for g in range(NG))
            ms = jax.lax.fori_loop(0, H - 1, lambda h, ms: block(h, h + 1, ms), ms)
            for g in range(NG):
                s_ref[g, 0:8, :] = ms[g]
            o_ref[0:8, 0:TQ] = (s_ref[0, 0:8, :] + ot_ref[z_ref[0], pl.ds(pl.multiple_of(z_ref[0], 8), 8), 0:1]
                                + bb_ref[pl.ds(pl.multiple_of(z_ref[0], 8), 8), 0:TQ]).astype(bf16)
            o_copy(0).start()
            o_copy(0).wait()
            return

        gw_copy = pltpu.make_async_copy(gw_hbm, gw_ref, sems.at[NR + 8])
        gw_copy.start()
        x_copy(0).start()
        if PRO == 0:
            order = [w_copy(2), x_copy(1), w_copy(1), w_copy(0)]
        else:
            order = [w_copy(0), w_copy(2), x_copy(1), w_copy(1)]
        for cp in order + [x_copy(r) for r in range(2, NR)] + late:
            cp.start()
        z_ref[0] = 0
        ot_ref[:, H * VROWS - 8:H * VROWS, :] = jnp.ones((S // LANE, 8, LANE), f32)

        lane = jax.lax.broadcasted_iota(jnp.int32, (RC // 2, LANE), 1)
        vrow = jax.lax.broadcasted_iota(jnp.int32, (8, RC), 0)

        def head_rows(t, h, fill):
            lo = DH * h + 16
            if lo + 8 <= D:
                tail = t[lo:lo + 8, :]
            else:
                tail = jnp.concatenate([t[lo:lo + 4, :], t[lo:lo + 4, :]], axis=0)
            return t[DH * h:DH * h + 16, :], jnp.where(vrow < 4, tail, fill)

        def k_proj(r):
            k = jnp.dot(x_ref[_ds(r, RC), :], wqkv_ref[1], preferred_element_type=f32)
            kp = pltpu.bitcast(k.astype(bf16), u32)
            CPR = RC // CK
            for h in range(H):
                b, t0 = divmod(DH * h, LANE)
                src = kp[:, b * LANE:(b + 1) * LANE]
                if t0 + DH > LANE:
                    src = jnp.where(lane >= t0, src, kp[:, (b + 1) * LANE:(b + 2) * LANE])
                if t0:
                    src = pltpu.roll(src, LANE - t0, 1)
                kb_ref[h, _ds(r, RC // 2), :] = src
                for cc in range(CPR):
                    kf = pltpu.bitcast(src[cc * CK // 2:cc * CK // 2 + RMAX * 4, :], bf16).astype(f32)
                    ko_ref[h, _ds(r * CPR + cc, RMAX * 8), :] = kf

        def run_linked(jobs, res):
            n = len(jobs)
            nt = res.shape[1] // LANE
            for k, job in enumerate(jobs):
                t = k * (nt - 1) * res.shape[0] // n
                ct, row = t // res.shape[0], t % res.shape[0] // 8 * 8
                job(res[row:row + 8, ct * LANE:(ct + 1) * LANE])

        GR = 32

        def gate_jobs(r):
            def job(i, link):
                rows = _ds(r * (RC // GR) + i, GR)
                xb = x_ref[rows, :]
                xp_ref[r * (RC // FB) + i * GR // FB, pl.ds(i * GR % FB // 2, GR // 2), 0:D] = after(
                    pltpu.bitcast(xb, u32), link)
                gw = after(bf_ref[8:16, D:2 * D], link)
                xt = xb.astype(f32).reshape(GR // 8, 8, D)
                gl = jnp.sum((xt * gw[None]).reshape(GR, D), axis=-1, keepdims=True)
                gb_ref[rows, :] = jnp.broadcast_to(jax.nn.sigmoid(gl), (GR, LANE))
            return [lambda link, i=i: job(i, link) for i in range(RC // GR)]

        def q_proj(r, jobs=()):
            cols = _ds(r, RC)
            q = jnp.dot(x_ref[cols, :], wqkv_ref[0], preferred_element_type=f32)
            run_linked(jobs, q)
            q = q * qscale
            qt = q.astype(bf16).astype(f32).T
            zero8 = jnp.zeros((8, RC), f32)
            for h in range(H):
                top, tail = head_rows(qt, h, 0.0)
                qt_ref[h, 0:16, cols] = top
                qt_ref[h, 16:24, cols] = tail
                q32 = jnp.concatenate([top, tail, zero8], axis=0).astype(bf16)
                qm_ref[h, :, cols] = pltpu.bitcast(q32, u32)

        def v_proj(r, jobs=()):
            cols = _ds(r, RC)
            v = jnp.dot(x_ref[cols, :], wqkv_ref[2], preferred_element_type=f32)
            run_linked(jobs, v)
            vt = v.T
            fill = jnp.where(vrow == 4, 1.0, 0.0)
            for h in range(H):
                top, tail = head_rows(vt, h, fill)
                vt_ref[h, 0:16, cols] = top
                vt_ref[h, 16:24, cols] = tail

        gw_copy.wait()
        bf_ref[8:16, D:2 * D] = jnp.broadcast_to(gw_ref[...].astype(f32)[None, :], (8, D))
        x_copy(0).wait()
        if PRO == 0:
            w_copy(2).wait()
            v_proj(0, gate_jobs(0))
            w_copy(1).wait()
            w_copy(0).wait()
        else:
            w_copy(0).wait()
            q_proj(0)
            w_copy(2).wait()
            v_proj(0, gate_jobs(0))
            w_copy(1).wait()

        def proj(r, _):
            x_copy(r + 1).wait()
            k_proj(r)
            q_proj(r + PRO, gate_jobs(r + 1))
            v_proj(r + 1)
            return 0
        jax.lax.fori_loop(0, NR - 1, proj, 0)
        for cp in late[:-1]:
            cp.wait()
        bf_ref[0:8, :] = jnp.broadcast_to(b1_ref[...].astype(f32)[None, :], (8, F))
        packs = ([(w1_ref, w1p_ref, i, 1) for i in range(D // 16)]
                 + [(w2_ref, w2p_ref, i, 3) for i in range(F // 48)]
                 + [(wo_ref, wop_ref, i, 2) for i in range(D // 32)])

        def pack_job(src, dst, i, n, link):
            dst[pl.ds(i * n * 8, n * 8), :] = after(pltpu.bitcast(src[pl.ds(i * n * 16, n * 16), :], u32), link)
        k_proj(NR - 1)
        q_proj(NR - 1, [lambda link, p=p: pack_job(*p, link) for p in packs])

        def side(u, link):
            if u >= NU - 2 * NV and (u - (NU - 2 * NV)) % 2 == 0:
                i = (u - (NU - 2 * NV)) // 2
                c = max(cc for cc in range(NC) if vstart[cc] <= i and rv[cc])
                make_kbc(1, c, i - vstart[c], link)
        ms = block(None, 0, None, extra=side, rvg=[[0] * NC] * NG)
        ms = jax.lax.fori_loop(0, H - 1, lambda h, ms: block(h, h + 1, ms), ms)
        late[-1].wait()
        for g in range(NG):
            m_ref[g] = ms[g]
        bf_ref[8:16, 0:D] = jnp.broadcast_to(b2_ref[...].astype(f32)[None, :], (8, D))

        K1 = (NKT - 1) * LANE

        def stage(g, first=False, last=False):
            base = g if first else g - 1
            n = 1 if (first or last) else 2
            cur = 0 if first else 1
            otv = ot_ref.at[pl.ds(base * NJ, n * NJ)]
            otcv = otc_ref.at[pl.ds(base * NJ, n * NJ)]
            invv = inv_ref.at[pl.ds(base * NJ, n * NJ)]
            opv = op_ref.at[pl.ds(base * NJ, n * NJ)]
            rows0 = base * TQ if isinstance(base, int) else pl.multiple_of(base * TQ, TQ)
            bbv = bb_ref.at[pl.ds(rows0, TQ)]
            gbv = gb_ref.at[pl.ds(rows0, TQ)]
            ov = o_ref.at[pl.ds(rows0, TQ)]

            def prep(t, h0, h1, k0, k1):
                for h in range(h0, h1):
                    otcv[t, DH * h:DH * h + DH, :] = otv[t, pl.ds(h * VROWS, DH), :] * invv[t, pl.ds(h, 1), :]
                o = otcv[t, k0 * LANE:k1 * LANE, :].T.astype(bf16)
                opv[t, :, k0 * LANE:k1 * LANE] = pltpu.bitcast(o, u32)

            def prep_early(j, link):
                t = cur * NJ + j
                den = otv[t, pl.ds(DH, H, stride=VROWS), :]
                invv[t] = 1.0 / (den if link is None else after(den, link))
                prep(t, 0, H - 1, 0, NKT - 1)

            def prep_late():
                for t in range(NJ):
                    invv[t, H - 1:H, :] = 1.0 / otv[t, pl.ds((H - 1) * VROWS + DH, 1), :]
                    prep(t, H - 1, H, NKT - 1, NKT)

            def a1(rt, ct):
                rows = pl.ds(rt * LANE, LANE)
                cols = pl.ds(ct * LANE, LANE)
                o = pltpu.bitcast(opv[rt, :, 0:K1], bf16)
                w = pltpu.bitcast(wop_ref[0:K1 // 2, cols], bf16)
                a = jnp.dot(o, w, preferred_element_type=f32)
                gt = gbv[rows, :]
                bbv[rows, cols] = gt * a + (1.0 - gt) * (bbv[rows, cols] + bf_ref[8:9, cols])

            def a2(ct):
                cols = pl.ds(ct * LANE, LANE)
                o = pltpu.bitcast(opv[0:NJ, :, K1:D].reshape(TQ // 2, LANE), bf16)
                w = pltpu.bitcast(wop_ref[K1 // 2:D // 2, cols], bf16)
                a = jnp.dot(o, w, preferred_element_type=f32)
                ov[:, cols] = (bbv[:, cols] + gbv[...] * a).astype(bf16)

            jobs = []
            if first:
                fst = {}
                jobs += [lambda fd=fd: ffn_dot(H - 1, fst, *fd, FR=FB) for fd in fdots if fd[1] == 0]
            else:
                jobs.append(prep_late)
                for ct in range(NKT):
                    jobs += [lambda rt=rt, ct=ct: a1(rt, ct) for rt in range(NJ)]
                    if ct > 0:
                        jobs.append(lambda ct=ct: a2(ct - 1))
                jobs.append(lambda: a2(NKT - 1))
            if last:
                for job in jobs:
                    job()
            else:
                m = m_ref[g]
                acc = None
                for c in range(NC):
                    for k, job in enumerate(jobs):
                        if k * NC // len(jobs) == c:
                            job()
                    if c in PREPC:
                        prep_early(list(PREPC).index(c), None if acc is None else acc[0:8, 0:LANE])
                    s = s_ref[g, pl.ds(c * CK, CK), :].reshape(G8, 8, TQ)
                    p = jnp.exp2(s - m[None]).reshape(CK, TQ)
                    pv = jnp.dot(vt_ref[H - 1, :, pl.ds(c * CK, CK)], p, preferred_element_type=f32)
                    acc = pv if c == 0 else pv + acc
                for j in range(NJ):
                    otv[cur * NJ + j, _ds(H - 1, VROWS), :] = acc[:, j * LANE:(j + 1) * LANE]
            if not first:
                o_copy(g - 1).start()

        stage(0, first=True)

        def tail(g, _):
            stage(g)
            return 0
        jax.lax.fori_loop(1, NG, tail, 0)
        stage(NG, last=True)
        for g in range(NG):
            o_copy(g).wait()

    spec = dict(
        x=pltpu.VMEM((S, D), bf16),
        wqkv=pltpu.VMEM((3, D, D), bf16),
        wo=pltpu.VMEM((D, D), bf16),
        w1=pltpu.VMEM((D, F), bf16),
        w2=pltpu.VMEM((F, D), bf16),
        sems=pltpu.SemaphoreType.DMA((NR + 9,)),
        kb=pltpu.VMEM((H, S // 2, LANE), u32),
        qm=pltpu.VMEM((H, KD // 2, S), u32),
        vt=pltpu.VMEM((H, VROWS, S), f32),
        s=pltpu.VMEM((NG, S, TQ), f32),
        ot=pltpu.VMEM((S // LANE, H * VROWS, LANE), f32),
        otc=pltpu.VMEM((S // LANE, D, LANE), f32),
        bb=pltpu.VMEM((S, D), f32),
        qt=pltpu.VMEM((H, VROWS, S), f32),
        kbc=pltpu.VMEM((max(NV, 1), DH, 8, LANE), f32),
        hid=pltpu.VMEM((FB // 2, F), u32),
        z=pltpu.SMEM((1,), jnp.int32),
        ko=pltpu.VMEM((H, NC * RMAX * 8, LANE), f32),
        w1p=pltpu.VMEM((D // 2, F), u32),
        w2p=pltpu.VMEM((F // 2, D), u32),
        wop=pltpu.VMEM((D // 2, D), u32),
        bf=pltpu.VMEM((16, F), f32),
        o=pltpu.VMEM((S, D), bf16),
        osems=pltpu.SemaphoreType.DMA((NG,)),
        m=pltpu.VMEM((NG, 8, TQ), f32),
        gb=pltpu.VMEM((S, LANE), f32),
        inv=pltpu.VMEM((S // LANE, H, LANE), f32),
        op=pltpu.VMEM((S // LANE, LANE // 2, D), u32),
        xp=pltpu.VMEM((H, FB // 2, XW), u32),
        b1=pltpu.VMEM((F,), bf16),
        b2=pltpu.VMEM((D,), bf16),
        gw=pltpu.VMEM((D,), bf16),
        pad=pltpu.VMEM((PAD * 8, LANE), f32),
    )
    names = list(ORDER.split())
    assert sorted(names) == sorted(spec)
    scratch = [spec[n] for n in names]
    inner = kernel
    canon = list(spec)

    def kernel(*refs):
        io, sc = refs[:9], dict(zip(names, refs[9:]))
        inner(*io, *[sc[n] for n in canon if n != 'pad'])
    return kernel, scratch


def build(TQ=512, CK=128, RC=512, RVG=("2" * 16,) * 3 + ("2220" * 4,), POFF=3, FR=32,
          FSKIP=(15, 31, 47, 63), ONLY=0, PRO=0, VL=110,
          PAD=7, XW=640, PREPC=(2, 5, 8, 11), ORDER="pad s kbc qt w1p w2p hid bf kb qm vt bb xp x ko ot m gb wop op inv o otc wqkv wo w1 w2 sems osems z b1 b2 gw"):
    kernel, scratch = make_kernel(TQ, CK, RC, RVG, POFF, FR, FSKIP, ONLY, PRO, ORDER, PAD, XW, PREPC)

    def fn(A_x, A_wqkv, A_wo, B_x, B_w1, B_b1, B_w2, B_b2, gate_w):
        x = A_x.reshape(S, D)
        hbm = pl.BlockSpec(memory_space=pl.ANY)
        out = pl.pallas_call(
            kernel,
            in_specs=[hbm] * 8,
            out_specs=hbm,
            out_shape=jax.ShapeDtypeStruct((S, D), bf16),
            scratch_shapes=scratch,
            compiler_params=pltpu.CompilerParams(vmem_limit_bytes=VL * 1024 * 1024),
        )(x, A_wqkv, A_wo, B_w1, B_b1, B_w2, B_b2, gate_w)
        return out.reshape(1, S, D)
    return fn


@jax.jit
def pallas_gated_mix__softmax_full_mha__dense_activation_squared_relu__prompt_kernel(
    A_x: jax.Array,
    A_wqkv: jax.Array,
    A_wo: jax.Array,
    B_x: jax.Array,
    B_w1: jax.Array,
    B_b1: jax.Array,
    B_w2: jax.Array,
    B_b2: jax.Array,
    gate_w: jax.Array,
):
    return build()(A_x, A_wqkv, A_wo, B_x, B_w1, B_b1, B_w2, B_b2, gate_w)
```

```python
import math

import jax
import jax.numpy as jnp
import jax.experimental.pallas as pl
import jax.experimental.pallas.tpu as pltpu

S = 2048
D = 640
H = 32
DH = 20
F = 1536
LANE = 128
VROWS = 24
KD = 32
NKT = D // LANE
TQ = 512
NG = S // TQ
NJ = TQ // LANE
CK = 128
NC = S // CK
G8 = CK // 8
NU = NG * NC
RC = 512
X0 = 256
FB = S // H
FR = 32
GR = 32
NLAST = 4
RV = 2
RVG = [[RV] * NC] * (NG - 1) + [[RV, RV, RV, 0] * (NC // 4)]
LAST_USE = {c: max(g for g in range(NG) if RVG[g][c]) for c in range(NC)}
POFF = 3
PREPC = (2, 5, 8, 11)
QSCALE = (DH ** -0.5) * math.log2(math.e)
FDOTS = [(ph, rp, th, sub) for ph in range(2) for rp in range(FB // FR) for th in range(3) for sub in range(NKT)]
FMAP = dict(zip([u for u in range(NU) if u % NC != NC - 1], FDOTS))

f32 = jnp.float32
bf16 = jnp.bfloat16
u32 = jnp.uint32


def _ds(i, n):
    return pl.ds(i * n, n) if isinstance(i, int) else pl.ds(pl.multiple_of(i * n, n), n)


def _kernel(x_hbm, wqkv_hbm, wo_hbm, w1_hbm, b1_hbm, w2_hbm, b2_hbm, gw_hbm, o_hbm,
            s_ref, kbc_ref, qt_ref, w1p_ref, w2p_ref, bf_ref, kb_ref, qm_ref, vt_ref, bb_ref, xp_ref, x_ref,
            ko_ref, ot_ref, m_ref, gb_ref, wop_ref, wvt_ref, op_ref, inv_ref, o_ref, otc_ref,
            wqkv_ref, wo_ref, w1_ref, w2_ref, sems, osems, z_ref, b1_ref, b2_ref, gw_ref):

    def x_copy(r):
        return pltpu.make_async_copy(x_hbm.at[_ds(r, RC), :], x_ref.at[_ds(r, RC), :], sems.at[r])

    def w_copy(p):
        return pltpu.make_async_copy(wqkv_hbm.at[:, pl.ds(p * D, D)], wqkv_ref.at[p], sems.at[4 + p])

    xa_copy = pltpu.make_async_copy(x_hbm.at[0:X0, :], x_ref.at[0:X0, :], sems.at[0])
    xb_copy = pltpu.make_async_copy(x_hbm.at[X0:2 * RC, :], x_ref.at[X0:2 * RC, :], sems.at[1])
    gw_copy = pltpu.make_async_copy(gw_hbm, gw_ref, sems.at[7])
    b2_copy = pltpu.make_async_copy(b2_hbm, b2_ref, sems.at[8])
    late = [pltpu.make_async_copy(w1_hbm, w1_ref, sems.at[9]),
            pltpu.make_async_copy(w2_hbm, w2_ref, sems.at[10]),
            pltpu.make_async_copy(wo_hbm, wo_ref, sems.at[11]),
            pltpu.make_async_copy(b1_hbm, b1_ref, sems.at[12])]

    def o_copy(g):
        return pltpu.make_async_copy(o_ref.at[_ds(g, TQ), :], o_hbm.at[_ds(g, TQ), :], osems.at[g])

    def last_copy(i):
        rows = pl.ds((NG - 1) * TQ + i * (TQ // NLAST), TQ // NLAST)
        return pltpu.make_async_copy(o_ref.at[rows, :], o_hbm.at[rows, :], osems.at[NG - 1 + i])

    def colmax8(s):
        return jnp.max(s.reshape(s.shape[0] // 8, 8, s.shape[1]), axis=0) if s.shape[0] > 8 else s

    def after(x, link):
        lk = link if x.dtype == f32 else pltpu.bitcast(link, x.dtype)
        lk = jnp.concatenate([lk] * (x.shape[1] // LANE), axis=1)
        lk = jnp.concatenate([lk] * (x.shape[0] // 8), axis=0)
        return jnp.where(jnp.full(x.shape, z_ref[0]) != 0, lk, x)

    def make_kbc(h, i, link=None):
        ko = ko_ref[h, pl.ds(i * 8, 8), :]
        if link is not None:
            ko = after(ko, link)
        for d in range(DH):
            kbc_ref[i, d] = jnp.broadcast_to(ko[:, d:d + 1], (8, LANE))

    def ffn_dot(fb, st, ph, rp, th, sub, fr=FR):
        hcols = slice(th * 512, (th + 1) * 512)
        if ph == 0:
            xt = pltpu.bitcast(xp_ref[fb, rp * fr // 2:(rp + 1) * fr // 2, sub * LANE:(sub + 1) * LANE], bf16)
            w = pltpu.bitcast(w1p_ref[sub * 64:(sub + 1) * 64, hcols], bf16)
            o = jnp.dot(xt, w, preferred_element_type=f32)
            st["a"] = o + (bf_ref[0:1, hcols] if sub == 0 else st["a"])
            if sub == NKT - 1:
                hid = jnp.maximum(st["a"], 0.0)
                st[rp, th] = (hid * hid).astype(bf16)
        else:
            r0 = fb * FB + rp * fr
            if not isinstance(r0, int):
                r0 = pl.multiple_of(r0, fr)
            w = pltpu.bitcast(w2p_ref[th * 256:(th + 1) * 256, sub * LANE:(sub + 1) * LANE], bf16)
            o = jnp.dot(st[rp, th], w, preferred_element_type=f32)
            dst = (pl.ds(r0, fr), pl.ds(sub * LANE, LANE))
            bb_ref[dst] = o if th == 0 else o + bb_ref[dst]

    def block(h, hn, ms):
        mnxt = []
        fst = {}
        if h is not None:
            hn2 = jnp.minimum(hn + 1, H - 1)

        def vpu_piece(g, c, r, j):
            i = c * RV + r

            def term(d):
                return kbc_ref[i, d] * qt_ref[hn, pl.ds(d, 1), pl.ds(g * TQ + j * LANE, LANE)]
            acc = jax.lax.fori_loop(1, DH, lambda d, a: a + term(d), term(0), unroll=True)
            s_ref[g, pl.ds((c * G8 + r) * 8, 8), pl.ds(j * LANE, LANE)] = acc
            if g == LAST_USE[c] and j == NJ - 1:
                make_kbc(hn2, i)
            return acc

        acc = None
        for u in range(NU):
            g, c = divmod(u, NC)
            if h is not None:
                s = s_ref[g, pl.ds(c * CK, CK), :].reshape(G8, 8, TQ)
                p = jnp.exp2(s - ms[g][None]).reshape(CK, TQ)
            if c == 0:
                cm = [None] * NJ
                queue = []
                taken = 0
                rv = RVG[g] if h is not None else [0] * NC
            queue += [(g, c, r, j) for r in range(rv[c]) for j in range(NJ)]
            n = min(sum(rv) * NJ * (c + 1) // NC - taken, len(queue))
            taken += n
            mine, queue = queue[:n], queue[n:]
            L = G8 - rv[c]
            kk = pltpu.bitcast(kb_ref[hn, pl.ds((c * G8 + rv[c]) * 4, L * 4), :], bf16)[:, 0:KD]
            qq = pltpu.bitcast(qm_ref[hn, :, pl.ds(g * TQ, TQ)], bf16)
            sn = jnp.dot(kk, qq, preferred_element_type=f32)
            s_ref[g, pl.ds((c * G8 + rv[c]) * 8, L * 8), :] = sn
            pos = [max(1, int(round((k + 1) / n * (L + POFF) - POFF))) for k in range(n)] + [L]
            done = 0
            for k in range(n + 1):
                if pos[k] > done:
                    lj = colmax8(sn[done * 8:pos[k] * 8, :])
                    for j in range(NJ):
                        x = lj[:, j * LANE:(j + 1) * LANE]
                        cm[j] = x if cm[j] is None else jnp.maximum(cm[j], x)
                    done = pos[k]
                if k < n:
                    j = mine[k][3]
                    cm[j] = jnp.maximum(cm[j], vpu_piece(*mine[k]))
            if c == NC - 1:
                assert not queue
                m = jnp.concatenate(cm, axis=1)
                mnxt.append(jnp.broadcast_to(jnp.max(m, axis=0, keepdims=True), (8, TQ)))
            if h is not None:
                pv = jnp.dot(vt_ref[h, :, pl.ds(c * CK, CK)], p, preferred_element_type=f32)
                acc = pv if c == 0 else pv + acc
                if c == NC - 1:
                    for j in range(NJ):
                        ot_ref[g * NJ + j, _ds(h, VROWS), :] = acc[:, j * LANE:(j + 1) * LANE]
                if u in FMAP:
                    ffn_dot(h, fst, *FMAP[u])
            elif u % 2 == 0:
                make_kbc(hn + 1, u // 2, sn[0:8, 0:LANE])
        return tuple(mnxt)

    for cp in [gw_copy, w_copy(2), xa_copy, xb_copy, w_copy(1), w_copy(0), x_copy(2), x_copy(3)] + late + [b2_copy]:
        cp.start()
    z_ref[0] = 0
    ot_ref[:, H * VROWS - 8:H * VROWS, :] = jnp.ones((S // LANE, 8, LANE), f32)

    lane = jax.lax.broadcasted_iota(jnp.int32, (RC // 2, LANE), 1)

    def head_rows(t, h, ones_row):
        vrow = jax.lax.broadcasted_iota(jnp.int32, (8, t.shape[1]), 0)
        lo = DH * h + 16
        if lo + 8 <= D:
            tail = t[lo:lo + 8, :]
        else:
            tail = jnp.concatenate([t[lo:lo + 4, :], t[lo:lo + 4, :]], axis=0)
        fill = jnp.where(vrow == 4, 1.0, 0.0) if ones_row else 0.0
        return t[DH * h:DH * h + 16, :], jnp.where(vrow < 4, tail, fill)

    def run_linked(jobs, res):
        nt = res.shape[1] // LANE
        for k, job in enumerate(jobs):
            t = k * (nt - 1) * res.shape[0] // len(jobs)
            ct, row = t // res.shape[0], t % res.shape[0] // 8 * 8
            job(res[row:row + 8, ct * LANE:(ct + 1) * LANE])

    def gate_jobs(r):
        def job(i, link):
            rows = _ds(r * (RC // GR) + i, GR)
            xb = x_ref[rows, :]
            xp_ref[r * (RC // FB) + i * GR // FB, pl.ds(i * GR % FB // 2, GR // 2), :] = after(
                pltpu.bitcast(xb, u32), link)
            gw = after(bf_ref[8:16, D:2 * D], link)
            xt = xb.astype(f32).reshape(GR // 8, 8, D)
            gl = jnp.sum((xt * gw[None]).reshape(GR, D), axis=-1, keepdims=True)
            gb_ref[rows, :] = jnp.broadcast_to(jax.nn.sigmoid(gl), (GR, LANE))
        return [lambda link, i=i: job(i, link) for i in range(RC // GR)]

    def k_proj(r, jobs=()):
        k = jnp.dot(x_ref[_ds(r, RC), :], wqkv_ref[1], preferred_element_type=f32)
        run_linked(jobs, k)
        kp = pltpu.bitcast(k.astype(bf16), u32)
        cpr = RC // CK
        for h in range(H):
            b, t0 = divmod(DH * h, LANE)
            src = kp[:, b * LANE:(b + 1) * LANE]
            if t0 + DH > LANE:
                src = jnp.where(lane >= t0, src, kp[:, (b + 1) * LANE:(b + 2) * LANE])
            if t0:
                src = pltpu.roll(src, LANE - t0, 1)
            kb_ref[h, _ds(r, RC // 2), :] = src
            for cc in range(cpr):
                kf = pltpu.bitcast(src[cc * CK // 2:cc * CK // 2 + RV * 4, :], bf16).astype(f32)
                ko_ref[h, _ds(r * cpr + cc, RV * 8), :] = kf

    def q_proj(r, jobs):
        cols = _ds(r, RC)
        qt = jax.lax.dot_general(wqkv_ref[0], x_ref[cols, :], (((0,), (1,)), ((), ())),
                                 preferred_element_type=f32)
        run_linked(jobs, qt)
        qt = (qt * QSCALE).astype(bf16).astype(f32)
        zero8 = jnp.zeros((8, RC), f32)
        for h in range(H):
            top, tail = head_rows(qt, h, False)
            qt_ref[h, 0:16, cols] = top
            qt_ref[h, 16:24, cols] = tail
            q32 = jnp.concatenate([top, tail, zero8], axis=0).astype(bf16)
            qm_ref[h, :, cols] = pltpu.bitcast(q32, u32)

    def v_proj(cols, split=1):
        xc = x_ref[cols, :]
        n = D // 2 // split
        vt = jnp.concatenate([
            jax.lax.dot_general(pltpu.bitcast(wvt_ref[i * n:(i + 1) * n, :], bf16), xc, (((1,), (1,)), ((), ())),
                                preferred_element_type=f32) for i in range(split)], axis=0)
        for h in range(H):
            top, tail = head_rows(vt, h, True)
            vt_ref[h, 0:16, cols] = top
            vt_ref[h, 16:24, cols] = tail

    gw_copy.wait()
    bf_ref[8:16, D:2 * D] = jnp.broadcast_to(gw_ref[...].astype(f32)[None, :], (8, D))
    w_copy(2).wait()
    wvt_ref[...] = pltpu.bitcast(wqkv_ref[2].T, u32)
    xa_copy.wait()
    v_proj(pl.ds(0, X0), 2)
    xb_copy.wait()
    v_proj(pl.ds(X0, RC - X0), 2)
    v_proj(_ds(1, RC))
    w_copy(1).wait()
    w_copy(0).wait()

    def proj(r, _):
        x_copy(r + 2).wait()
        k_proj(r, gate_jobs(r))
        q_proj(r, gate_jobs(r + 2))
        v_proj(_ds(r + 2, RC))
        return 0
    jax.lax.fori_loop(0, 2, proj, 0)
    for cp in late:
        cp.wait()
    bf_ref[0:8, :] = jnp.broadcast_to(b1_ref[...].astype(f32)[None, :], (8, F))

    def pack_job(src, dst, i, n, link):
        dst[pl.ds(i * n * 8, n * 8), :] = after(pltpu.bitcast(src[pl.ds(i * n * 16, n * 16), :], u32), link)
    packs = ([(w1_ref, w1p_ref, i, 1) for i in range(D // 16)]
             + [(w2_ref, w2p_ref, i, 3) for i in range(F // 48)]
             + [(wo_ref, wop_ref, i, 2) for i in range(D // 32)])
    pjobs = [lambda link, p=p: pack_job(*p, link) for p in packs]
    k_proj(2)
    q_proj(2, pjobs[:len(pjobs) // 2])
    k_proj(3)
    q_proj(3, pjobs[len(pjobs) // 2:])

    ms = block(None, 0, None)
    ms = jax.lax.fori_loop(0, H - 1, lambda h, ms: block(h, h + 1, ms), ms)
    b2_copy.wait()
    for g in range(NG):
        m_ref[g] = ms[g]
    bf_ref[8:16, 0:D] = jnp.broadcast_to(b2_ref[...].astype(f32)[None, :], (8, D))

    K1 = (NKT - 1) * LANE

    def stage(g, first=False, last=False):
        base = g if first else g - 1
        n = 1 if (first or last) else 2
        cur = 0 if first else 1
        otv = ot_ref.at[pl.ds(base * NJ, n * NJ)]
        otcv = otc_ref.at[pl.ds(base * NJ, n * NJ)]
        invv = inv_ref.at[pl.ds(base * NJ, n * NJ)]
        opv = op_ref.at[pl.ds(base * NJ, n * NJ)]
        bbv = bb_ref.at[_ds(base, TQ)]
        gbv = gb_ref.at[_ds(base, TQ)]
        ov = o_ref.at[_ds(base, TQ)]

        def prep(t, h0, h1, k0, k1):
            for h in range(h0, h1):
                otcv[t, DH * h:DH * h + DH, :] = otv[t, pl.ds(h * VROWS, DH), :] * invv[t, pl.ds(h, 1), :]
            o = otcv[t, k0 * LANE:k1 * LANE, :].T.astype(bf16)
            opv[t, :, k0 * LANE:k1 * LANE] = pltpu.bitcast(o, u32)

        def prep_early(j, link):
            t = cur * NJ + j
            invv[t] = 1.0 / after(otv[t, pl.ds(DH, H, stride=VROWS), :], link)
            prep(t, 0, H - 1, 0, NKT - 1)

        def prep_late():
            for t in range(NJ):
                invv[t, H - 1:H, :] = 1.0 / otv[t, pl.ds((H - 1) * VROWS + DH, 1), :]
                prep(t, H - 1, H, NKT - 1, NKT)

        def a1(rt, ct):
            rows = pl.ds(rt * LANE, LANE)
            cols = pl.ds(ct * LANE, LANE)
            o = pltpu.bitcast(opv[rt, :, 0:K1], bf16)
            w = pltpu.bitcast(wop_ref[0:K1 // 2, cols], bf16)
            a = jnp.dot(o, w, preferred_element_type=f32)
            gt = gbv[rows, :]
            bbv[rows, cols] = gt * a + (1.0 - gt) * (bbv[rows, cols] + bf_ref[8:9, cols])

        def a2(ct, t0, t1):
            rows = pl.ds(t0 * LANE, (t1 - t0) * LANE)
            cols = pl.ds(ct * LANE, LANE)
            o = pltpu.bitcast(opv[t0:t1, :, K1:D].reshape((t1 - t0) * LANE // 2, LANE), bf16)
            w = pltpu.bitcast(wop_ref[K1 // 2:D // 2, cols], bf16)
            a = jnp.dot(o, w, preferred_element_type=f32)
            ov[rows, cols] = (bbv[rows, cols] + gbv[rows, :] * a).astype(bf16)

        if last:
            prep_late()
            per = NJ // NLAST
            for i in range(NLAST):
                lag = 2 if i == 0 else 1
                for ct in range(NKT + lag):
                    if ct < NKT:
                        for rt in range(i * per, (i + 1) * per):
                            a1(rt, ct)
                    if ct >= lag:
                        a2(ct - lag, i * per, (i + 1) * per)
                last_copy(i).start()
            return

        if first:
            fst = {}
            jobs = [lambda fd=fd: ffn_dot(H - 1, fst, *fd, fr=FB) for fd in FDOTS if fd[1] == 0]
        else:
            jobs = [prep_late]
            for ct in range(NKT):
                jobs += [lambda rt=rt, ct=ct: a1(rt, ct) for rt in range(NJ)]
                if ct > 0:
                    jobs.append(lambda ct=ct: a2(ct - 1, 0, NJ))
            jobs.append(lambda: a2(NKT - 1, 0, NJ))
        m = m_ref[g]
        acc = None
        for c in range(NC):
            for k, job in enumerate(jobs):
                if k * NC // len(jobs) == c:
                    job()
            if c in PREPC:
                prep_early(PREPC.index(c), acc[0:8, 0:LANE])
            s = s_ref[g, pl.ds(c * CK, CK), :].reshape(G8, 8, TQ)
            p = jnp.exp2(s - m[None]).reshape(CK, TQ)
            pv = jnp.dot(vt_ref[H - 1, :, pl.ds(c * CK, CK)], p, preferred_element_type=f32)
            acc = pv if c == 0 else pv + acc
        for j in range(NJ):
            otv[cur * NJ + j, _ds(H - 1, VROWS), :] = acc[:, j * LANE:(j + 1) * LANE]
        if not first:
            o_copy(g - 1).start()

    stage(0, first=True)

    def tail(g, _):
        stage(g)
        return 0
    jax.lax.fori_loop(1, NG, tail, 0)
    stage(NG, last=True)
    for g in range(NG - 1):
        o_copy(g).wait()
    for i in range(NLAST):
        last_copy(i).wait()


_SCRATCH = [
    pltpu.VMEM((NG, S, TQ), f32),
    pltpu.VMEM((NC * RV, DH, 8, LANE), f32),
    pltpu.VMEM((H, VROWS, S), f32),
    pltpu.VMEM((D // 2, F), u32),
    pltpu.VMEM((F // 2, D), u32),
    pltpu.VMEM((16, F), f32),
    pltpu.VMEM((H, S // 2, LANE), u32),
    pltpu.VMEM((H, KD // 2, S), u32),
    pltpu.VMEM((H, VROWS, S), f32),
    pltpu.VMEM((S, D), f32),
    pltpu.VMEM((H, FB // 2, D), u32),
    pltpu.VMEM((S, D), bf16),
    pltpu.VMEM((H, NC * RV * 8, LANE), f32),
    pltpu.VMEM((S // LANE, (H + 1) * VROWS, LANE), f32),
    pltpu.VMEM((NG, 8, TQ), f32),
    pltpu.VMEM((S, LANE), f32),
    pltpu.VMEM((D // 2, D), u32),
    pltpu.VMEM((D // 2, D), u32),
    pltpu.VMEM((S // LANE, LANE // 2, D), u32),
    pltpu.VMEM((S // LANE, H, LANE), f32),
    pltpu.VMEM((S, D), bf16),
    pltpu.VMEM((S // LANE, D, LANE), f32),
    pltpu.VMEM((3, D, D), bf16),
    pltpu.VMEM((D, D), bf16),
    pltpu.VMEM((D, F), bf16),
    pltpu.VMEM((F, D), bf16),
    pltpu.SemaphoreType.DMA((13,)),
    pltpu.SemaphoreType.DMA((NG - 1 + NLAST,)),
    pltpu.SMEM((1,), jnp.int32),
    pltpu.VMEM((F,), bf16),
    pltpu.VMEM((D,), bf16),
    pltpu.VMEM((D,), bf16),
]


@jax.jit
def pallas_gated_mix__softmax_full_mha__dense_activation_squared_relu__prompt_kernel(
    A_x: jax.Array,
    A_wqkv: jax.Array,
    A_wo: jax.Array,
    B_x: jax.Array,
    B_w1: jax.Array,
    B_b1: jax.Array,
    B_w2: jax.Array,
    B_b2: jax.Array,
    gate_w: jax.Array,
):
    del B_x
    hbm = pl.BlockSpec(memory_space=pl.ANY)
    out = pl.pallas_call(
        _kernel,
        in_specs=[hbm] * 8,
        out_specs=hbm,
        out_shape=jax.ShapeDtypeStruct((S, D), bf16),
        scratch_shapes=_SCRATCH,
        compiler_params=pltpu.CompilerParams(vmem_limit_bytes=110 * 1024 * 1024),
    )(A_x.reshape(S, D), A_wqkv, A_wo, B_w1, B_b1, B_w2, B_b2, gate_w)
    return out.reshape(1, S, D)
```

```python
import math

import jax
import jax.numpy as jnp
import jax.experimental.pallas as pl
import jax.experimental.pallas.tpu as pltpu

S = 2048
D = 640
H = 32
DH = 20
F = 1536
LANE = 128
VROWS = 24
KD = 32
NKT = D // LANE
TQ = 512
NG = S // TQ
NJ = TQ // LANE
CK = 128
NC = S // CK
G8 = CK // 8
NU = NG * NC
RC = 512
X0 = 256
FB = S // H
FR = 32
GR = 32
NLAST = 4
RV = 2
RVG = [[RV] * NC] * (NG - 1) + [[RV, RV, RV, 0] * (NC // 4)]
LAST_USE = {c: max(g for g in range(NG) if RVG[g][c]) for c in range(NC)}
POFF = 3
PREPC = (1, 3, 5, 7)
QSCALE = (DH ** -0.5) * math.log2(math.e)
FDOTS = [(ph, rp, th, sub) for ph in range(2) for rp in range(FB // FR) for th in range(3) for sub in range(NKT)]
FMAP = dict(zip([u for u in range(NU) if u % NC != NC - 1], FDOTS))

f32 = jnp.float32
bf16 = jnp.bfloat16
u32 = jnp.uint32


def _ds(i, n):
    return pl.ds(i * n, n) if isinstance(i, int) else pl.ds(pl.multiple_of(i * n, n), n)


def _kernel(x_hbm, wqkv_hbm, wo_hbm, w1_hbm, b1_hbm, w2_hbm, b2_hbm, gw_hbm, o_hbm,
            s_ref, kbc_ref, qt_ref, w1p_ref, w2p_ref, bf_ref, kb_ref, qm_ref, vt_ref, bb_ref, xp_ref, x_ref,
            ko_ref, ot_ref, m_ref, gb_ref, wop_ref, wvt_ref, op_ref, inv_ref, o_ref,
            wqkv_ref, wo_ref, w1_ref, w2_ref, sems, z_ref, b1_ref, b2_ref, gw_ref):

    def x_copy(r):
        return pltpu.make_async_copy(x_hbm.at[_ds(r, RC), :], x_ref.at[_ds(r, RC), :], sems.at[r])

    def w_copy(p):
        return pltpu.make_async_copy(wqkv_hbm.at[:, pl.ds(p * D, D)], wqkv_ref.at[p], sems.at[4 + p // 2])

    xa_copy = pltpu.make_async_copy(x_hbm.at[0:X0, :], x_ref.at[0:X0, :], sems.at[0])
    xb_copy = pltpu.make_async_copy(x_hbm.at[X0:2 * RC, :], x_ref.at[X0:2 * RC, :], sems.at[1])
    gw_copy = pltpu.make_async_copy(gw_hbm, gw_ref, sems.at[6])
    b2_copy = pltpu.make_async_copy(b2_hbm, b2_ref, sems.at[7])
    late = [pltpu.make_async_copy(w1_hbm, w1_ref, sems.at[8]),
            pltpu.make_async_copy(w2_hbm, w2_ref, sems.at[8]),
            pltpu.make_async_copy(wo_hbm, wo_ref, sems.at[8]),
            pltpu.make_async_copy(b1_hbm, b1_ref, sems.at[8])]

    def o_copy(g):
        return pltpu.make_async_copy(o_ref.at[_ds(g, TQ), :], o_hbm.at[_ds(g, TQ), :], sems.at[9])

    def last_copy(i):
        rows = pl.ds((NG - 1) * TQ + i * (TQ // NLAST), TQ // NLAST)
        return pltpu.make_async_copy(o_ref.at[rows, :], o_hbm.at[rows, :], sems.at[9])

    def colmax8(s):
        return jnp.max(s.reshape(s.shape[0] // 8, 8, s.shape[1]), axis=0) if s.shape[0] > 8 else s

    def after(x, link):
        lk = link if x.dtype == f32 else pltpu.bitcast(link, x.dtype)
        lk = jnp.concatenate([lk] * (x.shape[1] // LANE), axis=1)
        lk = jnp.concatenate([lk] * (x.shape[0] // 8), axis=0)
        return jnp.where(jnp.full(x.shape, z_ref[0]) != 0, lk, x)

    def make_kbc(h, i, link=None):
        ko = ko_ref[h, pl.ds(i * 8, 8), :]
        if link is not None:
            ko = after(ko, link)
        for d in range(DH):
            kbc_ref[i, d] = jnp.broadcast_to(ko[:, d:d + 1], (8, LANE))

    def ffn_dot(fb, st, ph, rp, th, sub, fr=FR):
        hcols = slice(th * 512, (th + 1) * 512)
        if ph == 0:
            xt = pltpu.bitcast(xp_ref[fb, rp * fr // 2:(rp + 1) * fr // 2, sub * LANE:(sub + 1) * LANE], bf16)
            w = pltpu.bitcast(w1p_ref[sub * 64:(sub + 1) * 64, hcols], bf16)
            o = jnp.dot(xt, w, preferred_element_type=f32)
            st["a"] = o + (bf_ref[0:1, hcols] if sub == 0 else st["a"])
            if sub == NKT - 1:
                hid = jnp.maximum(st["a"], 0.0)
                st[rp, th] = (hid * hid).astype(bf16)
        else:
            r0 = fb * FB + rp * fr
            if not isinstance(r0, int):
                r0 = pl.multiple_of(r0, fr)
            w = pltpu.bitcast(w2p_ref[th * 256:(th + 1) * 256, sub * LANE:(sub + 1) * LANE], bf16)
            o = jnp.dot(st[rp, th], w, preferred_element_type=f32)
            dst = (pl.ds(r0, fr), pl.ds(sub * LANE, LANE))
            bb_ref[dst] = o if th == 0 else o + bb_ref[dst]

    def block(h, hn, ms):
        mnxt = []
        fst = {}
        if h is not None:
            hn2 = jnp.minimum(hn + 1, H - 1)

        def vpu_piece(g, c, r, j):
            i = c * RV + r

            def term(d):
                return kbc_ref[i, d] * qt_ref[hn, pl.ds(d, 1), pl.ds(g * TQ + j * LANE, LANE)]
            acc = jax.lax.fori_loop(1, DH, lambda d, a: a + term(d), term(0), unroll=True)
            s_ref[g, pl.ds((c * G8 + r) * 8, 8), pl.ds(j * LANE, LANE)] = acc
            if g == LAST_USE[c] and j == NJ - 1:
                make_kbc(hn2, i)
            return acc

        acc = None
        for u in range(NU):
            g, c = divmod(u, NC)
            if h is not None:
                s = s_ref[g, pl.ds(c * CK, CK), :].reshape(G8, 8, TQ)
                p = jnp.exp2(s - ms[g][None]).reshape(CK, TQ)
            if c == 0:
                cm = [None] * NJ
                queue = []
                taken = 0
                rv = RVG[g] if h is not None else [0] * NC
            queue += [(g, c, r, j) for r in range(rv[c]) for j in range(NJ)]
            n = min(sum(rv) * NJ * (c + 1) // NC - taken, len(queue))
            taken += n
            mine, queue = queue[:n], queue[n:]
            L = G8 - rv[c]
            kk = pltpu.bitcast(kb_ref[hn, pl.ds((c * G8 + rv[c]) * 4, L * 4), :], bf16)[:, 0:KD]
            qq = pltpu.bitcast(qm_ref[hn, :, pl.ds(g * TQ, TQ)], bf16)
            sn = jnp.dot(kk, qq, preferred_element_type=f32)
            s_ref[g, pl.ds((c * G8 + rv[c]) * 8, L * 8), :] = sn
            pos = [max(1, int(round((k + 1) / n * (L + POFF) - POFF))) for k in range(n)] + [L]
            done = 0
            for k in range(n + 1):
                if pos[k] > done:
                    lj = colmax8(sn[done * 8:pos[k] * 8, :])
                    for j in range(NJ):
                        x = lj[:, j * LANE:(j + 1) * LANE]
                        cm[j] = x if cm[j] is None else jnp.maximum(cm[j], x)
                    done = pos[k]
                if k < n:
                    j = mine[k][3]
                    cm[j] = jnp.maximum(cm[j], vpu_piece(*mine[k]))
            if c == NC - 1:
                assert not queue
                m = jnp.concatenate(cm, axis=1)
                mnxt.append(jnp.broadcast_to(jnp.max(m, axis=0, keepdims=True), (8, TQ)))
            if h is not None:
                pv = jnp.dot(vt_ref[h, :, pl.ds(c * CK, CK)], p, preferred_element_type=f32)
                acc = pv if c == 0 else pv + acc
                if c == NC - 1:
                    for j in range(NJ):
                        ot_ref[g * NJ + j, _ds(h, VROWS), :] = acc[:, j * LANE:(j + 1) * LANE]
                if u in FMAP:
                    ffn_dot(h, fst, *FMAP[u])
            elif u % 2 == 0:
                make_kbc(hn + 1, u // 2, sn[0:8, 0:LANE])
        return tuple(mnxt)

    for cp in [gw_copy, w_copy(2), xa_copy, xb_copy, w_copy(1), w_copy(0), x_copy(2), x_copy(3)] + late + [b2_copy]:
        cp.start()
    z_ref[0] = 0
    ot_ref[:, H * VROWS - 8:H * VROWS, :] = jnp.ones((S // LANE, 8, LANE), f32)

    lane = jax.lax.broadcasted_iota(jnp.int32, (RC // 2, LANE), 1)

    def head_rows(t, h, ones_row):
        vrow = jax.lax.broadcasted_iota(jnp.int32, (8, t.shape[1]), 0)
        lo = DH * h + 16
        if lo + 8 <= D:
            tail = t[lo:lo + 8, :]
        else:
            tail = jnp.concatenate([t[lo:lo + 4, :], t[lo:lo + 4, :]], axis=0)
        fill = jnp.where(vrow == 4, 1.0, 0.0) if ones_row else 0.0
        return t[DH * h:DH * h + 16, :], jnp.where(vrow < 4, tail, fill)

    def run_linked(jobs, res):
        nt = res.shape[1] // LANE
        for k, job in enumerate(jobs):
            t = k * (nt - 1) * res.shape[0] // len(jobs)
            ct, row = t // res.shape[0], t % res.shape[0] // 8 * 8
            job(res[row:row + 8, ct * LANE:(ct + 1) * LANE])

    def gate_jobs(r):
        def job(i, link):
            rows = _ds(r * (RC // GR) + i, GR)
            xb = x_ref[rows, :]
            xp_ref[r * (RC // FB) + i * GR // FB, pl.ds(i * GR % FB // 2, GR // 2), :] = after(
                pltpu.bitcast(xb, u32), link)
            gw = after(bf_ref[8:16, D:2 * D], link)
            xt = xb.astype(f32).reshape(GR // 8, 8, D)
            gl = jnp.sum((xt * gw[None]).reshape(GR, D), axis=-1, keepdims=True)
            gb_ref[rows, :] = jnp.broadcast_to(jax.nn.sigmoid(gl), (GR, LANE))
        return [lambda link, i=i: job(i, link) for i in range(RC // GR)]

    def k_proj(r, jobs=()):
        k = jnp.dot(x_ref[_ds(r, RC), :], wqkv_ref[1], preferred_element_type=f32)
        run_linked(jobs, k)
        kp = pltpu.bitcast(k.astype(bf16), u32)
        cpr = RC // CK
        for h in range(H):
            b, t0 = divmod(DH * h, LANE)
            src = kp[:, b * LANE:(b + 1) * LANE]
            if t0 + DH > LANE:
                src = jnp.where(lane >= t0, src, kp[:, (b + 1) * LANE:(b + 2) * LANE])
            if t0:
                src = pltpu.roll(src, LANE - t0, 1)
            kb_ref[h, _ds(r, RC // 2), :] = src
            for cc in range(cpr):
                kf = pltpu.bitcast(src[cc * CK // 2:cc * CK // 2 + RV * 4, :], bf16).astype(f32)
                ko_ref[h, _ds(r * cpr + cc, RV * 8), :] = kf

    def q_proj(r, jobs):
        cols = _ds(r, RC)
        qt = jax.lax.dot_general(wqkv_ref[0], x_ref[cols, :], (((0,), (1,)), ((), ())),
                                 preferred_element_type=f32)
        run_linked(jobs, qt)
        qt = (qt * QSCALE).astype(bf16).astype(f32)
        zero8 = jnp.zeros((8, RC), f32)
        for h in range(H):
            top, tail = head_rows(qt, h, False)
            qt_ref[h, 0:16, cols] = top
            qt_ref[h, 16:24, cols] = tail
            q32 = jnp.concatenate([top, tail, zero8], axis=0).astype(bf16)
            qm_ref[h, :, cols] = pltpu.bitcast(q32, u32)

    def v_proj(cols, split=1):
        xc = x_ref[cols, :]
        n = D // 2 // split
        vt = jnp.concatenate([
            jax.lax.dot_general(pltpu.bitcast(wvt_ref[i * n:(i + 1) * n, :], bf16), xc, (((1,), (1,)), ((), ())),
                                preferred_element_type=f32) for i in range(split)], axis=0)
        for h in range(H):
            top, tail = head_rows(vt, h, True)
            vt_ref[h, 0:16, cols] = top
            vt_ref[h, 16:24, cols] = tail

    gw_copy.wait()
    bf_ref[8:16, D:2 * D] = jnp.broadcast_to(gw_ref[...].astype(f32)[None, :], (8, D))
    w_copy(2).wait()
    wvt_ref[...] = pltpu.bitcast(wqkv_ref[2].T, u32)
    xa_copy.wait()
    v_proj(pl.ds(0, X0), 2)
    xb_copy.wait()
    v_proj(pl.ds(X0, RC - X0), 2)
    v_proj(_ds(1, RC))
    w_copy(1).wait()
    w_copy(0).wait()

    def proj(r, _):
        x_copy(r + 2).wait()
        k_proj(r, gate_jobs(r))
        q_proj(r, gate_jobs(r + 2))
        v_proj(_ds(r + 2, RC))
        return 0
    jax.lax.fori_loop(0, 2, proj, 0)
    for cp in late:
        cp.wait()
    bf_ref[0:8, :] = jnp.broadcast_to(b1_ref[...].astype(f32)[None, :], (8, F))

    def pack_job(src, dst, i, n, link):
        dst[pl.ds(i * n * 8, n * 8), :] = after(pltpu.bitcast(src[pl.ds(i * n * 16, n * 16), :], u32), link)
    packs = ([(w1_ref, w1p_ref, i, 1) for i in range(D // 16)]
             + [(w2_ref, w2p_ref, i, 3) for i in range(F // 48)]
             + [(wo_ref, wop_ref, i, 2) for i in range(D // 32)])
    pjobs = [lambda link, p=p: pack_job(*p, link) for p in packs]
    k_proj(2)
    q_proj(2, pjobs[:len(pjobs) // 2])
    k_proj(3)
    q_proj(3, pjobs[len(pjobs) // 2:])

    ms = block(None, 0, None)
    ms = jax.lax.fori_loop(0, H - 1, lambda h, ms: block(h, h + 1, ms), ms)
    b2_copy.wait()
    for g in range(NG):
        m_ref[g] = ms[g]
    bf_ref[8:16, 0:D] = jnp.broadcast_to(b2_ref[...].astype(f32)[None, :], (8, D))

    K1 = (NKT - 1) * LANE

    def stage(g, first=False, last=False):
        base = g if first else g - 1
        n = 1 if (first or last) else 2
        cur = 0 if first else 1
        otv = ot_ref.at[pl.ds(base * NJ, n * NJ)]
        invv = inv_ref.at[pl.ds(base * NJ, n * NJ)]
        opv = op_ref.at[pl.ds(base * NJ, n * NJ)]
        bbv = bb_ref.at[_ds(base, TQ)]
        gbv = gb_ref.at[_ds(base, TQ)]
        ov = o_ref.at[_ds(base, TQ)]

        def prep(t, k0, k1):
            h0, h1 = k0 * LANE // DH, -(-k1 * LANE // DH)
            o = jnp.concatenate([otv[t, pl.ds(h * VROWS, DH), :] * invv[t, pl.ds(h, 1), :] for h in range(h0, h1)],
                                axis=0)[k0 * LANE - h0 * DH:k1 * LANE - h0 * DH, :]
            opv[t, :, k0 * LANE:k1 * LANE] = pltpu.bitcast(o.T.astype(bf16), u32)

        def prep_early(j, link):
            t = cur * NJ + j
            invv[t] = 1.0 / after(otv[t, pl.ds(DH, H, stride=VROWS), :], link)
            prep(t, 0, NKT - 1)

        def prep_late():
            for t in range(NJ):
                invv[t, H - 1:H, :] = 1.0 / otv[t, pl.ds((H - 1) * VROWS + DH, 1), :]
                prep(t, NKT - 1, NKT)

        def a1(rt, ct):
            rows = pl.ds(rt * LANE, LANE)
            cols = pl.ds(ct * LANE, LANE)
            o = pltpu.bitcast(opv[rt, :, 0:K1], bf16)
            w = pltpu.bitcast(wop_ref[0:K1 // 2, cols], bf16)
            a = jnp.dot(o, w, preferred_element_type=f32)
            gt = gbv[rows, :]
            bbv[rows, cols] = gt * a + (1.0 - gt) * (bbv[rows, cols] + bf_ref[8:9, cols])

        def a2(ct, t0, t1):
            rows = pl.ds(t0 * LANE, (t1 - t0) * LANE)
            cols = pl.ds(ct * LANE, LANE)
            o = pltpu.bitcast(opv[t0:t1, :, K1:D].reshape((t1 - t0) * LANE // 2, LANE), bf16)
            w = pltpu.bitcast(wop_ref[K1 // 2:D // 2, cols], bf16)
            a = jnp.dot(o, w, preferred_element_type=f32)
            ov[rows, cols] = (bbv[rows, cols] + gbv[rows, :] * a).astype(bf16)

        if last:
            prep_late()
            per = NJ // NLAST
            for i in range(NLAST):
                lag = 2 if i == 0 else 1
                for ct in range(NKT + lag):
                    if ct < NKT:
                        for rt in range(i * per, (i + 1) * per):
                            a1(rt, ct)
                    if ct >= lag:
                        a2(ct - lag, i * per, (i + 1) * per)
                last_copy(i).start()
            return

        if first:
            fst = {}
            jobs = [lambda fd=fd: ffn_dot(H - 1, fst, *fd, fr=FB) for fd in FDOTS if fd[1] == 0]
        else:
            jobs = [prep_late]
            for ct in range(NKT):
                jobs += [lambda rt=rt, ct=ct: a1(rt, ct) for rt in range(NJ)]
                if ct > 0:
                    jobs.append(lambda ct=ct: a2(ct - 1, 0, NJ))
            jobs.append(lambda: a2(NKT - 1, 0, NJ))
        m = m_ref[g]
        acc = None
        for c in range(NC):
            for k, job in enumerate(jobs):
                if k * NC // len(jobs) == c:
                    job()
            if c in PREPC:
                prep_early(PREPC.index(c), acc[0:8, 0:LANE])
            s = s_ref[g, pl.ds(c * CK, CK), :].reshape(G8, 8, TQ)
            p = jnp.exp2(s - m[None]).reshape(CK, TQ)
            pv = jnp.dot(vt_ref[H - 1, :, pl.ds(c * CK, CK)], p, preferred_element_type=f32)
            acc = pv if c == 0 else pv + acc
        for j in range(NJ):
            otv[cur * NJ + j, _ds(H - 1, VROWS), :] = acc[:, j * LANE:(j + 1) * LANE]
        if not first:
            o_copy(g - 1).start()

    stage(0, first=True)

    def tail(g, _):
        stage(g)
        return 0
    jax.lax.fori_loop(1, NG, tail, 0)
    stage(NG, last=True)
    for g in range(NG - 1):
        o_copy(g).wait()
    for i in range(NLAST):
        last_copy(i).wait()


_SCRATCH = [
    pltpu.VMEM((NG, S, TQ), f32),
    pltpu.VMEM((NC * RV, DH, 8, LANE), f32),
    pltpu.VMEM((H, VROWS, S), f32),
    pltpu.VMEM((D // 2, F), u32),
    pltpu.VMEM((F // 2, D), u32),
    pltpu.VMEM((16, F), f32),
    pltpu.VMEM((H, S // 2, LANE), u32),
    pltpu.VMEM((H, KD // 2, S), u32),
    pltpu.VMEM((H, VROWS, S), f32),
    pltpu.VMEM((S, D), f32),
    pltpu.VMEM((H, FB // 2, D), u32),
    pltpu.VMEM((S, D), bf16),
    pltpu.VMEM((H, NC * RV * 8, LANE), f32),
    pltpu.VMEM((S // LANE, (H + 1) * VROWS, LANE), f32),
    pltpu.VMEM((NG, 8, TQ), f32),
    pltpu.VMEM((S, LANE), f32),
    pltpu.VMEM((D // 2, D), u32),
    pltpu.VMEM((D // 2, D), u32),
    pltpu.VMEM((S // LANE, LANE // 2, D), u32),
    pltpu.VMEM((S // LANE, H, LANE), f32),
    pltpu.VMEM((S, D), bf16),
    pltpu.VMEM((3, D, D), bf16),
    pltpu.VMEM((D, D), bf16),
    pltpu.VMEM((D, F), bf16),
    pltpu.VMEM((F, D), bf16),
    pltpu.SemaphoreType.DMA((10,)),
    pltpu.SMEM((1,), jnp.int32),
    pltpu.VMEM((F,), bf16),
    pltpu.VMEM((D,), bf16),
    pltpu.VMEM((D,), bf16),
]


@jax.jit
def pallas_gated_mix__softmax_full_mha__dense_activation_squared_relu__prompt_kernel(
    A_x: jax.Array,
    A_wqkv: jax.Array,
    A_wo: jax.Array,
    B_x: jax.Array,
    B_w1: jax.Array,
    B_b1: jax.Array,
    B_w2: jax.Array,
    B_b2: jax.Array,
    gate_w: jax.Array,
):
    del B_x
    hbm = pl.BlockSpec(memory_space=pl.ANY)
    out = pl.pallas_call(
        _kernel,
        in_specs=[hbm] * 8,
        out_specs=hbm,
        out_shape=jax.ShapeDtypeStruct((S, D), bf16),
        scratch_shapes=_SCRATCH,
        compiler_params=pltpu.CompilerParams(vmem_limit_bytes=110 * 1024 * 1024),
    )(A_x.reshape(S, D), A_wqkv, A_wo, B_w1, B_b1, B_w2, B_b2, gate_w)
    return out.reshape(1, S, D)
```

```python
import math

import jax
import jax.numpy as jnp
import jax.experimental.pallas as pl
import jax.experimental.pallas.tpu as pltpu

S = 2048
D = 640
H = 32
DH = 20
F = 1536
LANE = 128
VROWS = 24
KD = 32
NKT = D // LANE
TQ = 512
NG = S // TQ
NJ = TQ // LANE
CK = 128
NC = S // CK
G8 = CK // 8
NU = NG * NC
RC = 512
X0 = 256
FB = S // H
FR = 32
GR = 32
NLAST = 4
RV = 2
RVG = [[RV] * NC] * (NG - 1) + [[RV] * (NC - 1) + [0]]
NPIECE = [[RV * NJ] * NC] * (NG - 1) + [[8, 8, 8, 8, 8, 8, 8, 8, 8, 8, 8, 6, 8, 6, 6, 6]]
LAST_USE = {c: max(g for g in range(NG) if RVG[g][c]) for c in range(NC)}
POFF = 3
PREPC = (1, 3, 5, 7)
QSCALE = (DH ** -0.5) * math.log2(math.e)
FDOTS = [(ph, rp, th, sub) for ph in range(2) for rp in range(FB // FR) for th in range(3) for sub in range(NKT)]
FMAP = dict(zip([u for u in range(NU) if u % NC != NC - 1], FDOTS))

f32 = jnp.float32
bf16 = jnp.bfloat16
u32 = jnp.uint32


def _ds(i, n):
    return pl.ds(i * n, n) if isinstance(i, int) else pl.ds(pl.multiple_of(i * n, n), n)


def _kernel(x_hbm, wqkv_hbm, wo_hbm, w1_hbm, b1_hbm, w2_hbm, b2_hbm, gw_hbm, o_hbm,
            s_ref, kbc_ref, qt_ref, w1p_ref, w2p_ref, bf_ref, kb_ref, qm_ref, vt_ref, bb_ref, xp_ref, x_ref,
            ko_ref, ot_ref, m_ref, gb_ref, wop_ref, wvt_ref, op_ref, inv_ref, o_ref,
            wqkv_ref, wo_ref, w1_ref, w2_ref, sems, z_ref, b1_ref, b2_ref, gw_ref):

    def x_copy(r):
        return pltpu.make_async_copy(x_hbm.at[_ds(r, RC), :], x_ref.at[_ds(r, RC), :], sems.at[r])

    def w_copy(p):
        return pltpu.make_async_copy(wqkv_hbm.at[:, pl.ds(p * D, D)], wqkv_ref.at[p], sems.at[4 + p // 2])

    xa_copy = pltpu.make_async_copy(x_hbm.at[0:X0, :], x_ref.at[0:X0, :], sems.at[0])
    xb_copy = pltpu.make_async_copy(x_hbm.at[X0:2 * RC, :], x_ref.at[X0:2 * RC, :], sems.at[1])
    gw_copy = pltpu.make_async_copy(gw_hbm, gw_ref, sems.at[6])
    b2_copy = pltpu.make_async_copy(b2_hbm, b2_ref, sems.at[7])
    late = [pltpu.make_async_copy(w1_hbm, w1_ref, sems.at[8]),
            pltpu.make_async_copy(w2_hbm, w2_ref, sems.at[8]),
            pltpu.make_async_copy(wo_hbm, wo_ref, sems.at[8]),
            pltpu.make_async_copy(b1_hbm, b1_ref, sems.at[8])]

    def o_copy(g):
        return pltpu.make_async_copy(o_ref.at[_ds(g, TQ), :], o_hbm.at[_ds(g, TQ), :], sems.at[9])

    def last_copy(i):
        rows = pl.ds((NG - 1) * TQ + i * (TQ // NLAST), TQ // NLAST)
        return pltpu.make_async_copy(o_ref.at[rows, :], o_hbm.at[rows, :], sems.at[9])

    def colmax8(s):
        return jnp.max(s.reshape(s.shape[0] // 8, 8, s.shape[1]), axis=0) if s.shape[0] > 8 else s

    def after(x, link):
        lk = link if x.dtype == f32 else pltpu.bitcast(link, x.dtype)
        lk = jnp.concatenate([lk] * (x.shape[1] // LANE), axis=1)
        lk = jnp.concatenate([lk] * (x.shape[0] // 8), axis=0)
        return jnp.where(jnp.full(x.shape, z_ref[0]) != 0, lk, x)

    def make_kbc(h, i, link=None):
        ko = ko_ref[h, pl.ds(i * 8, 8), :]
        if link is not None:
            ko = after(ko, link)
        cols = [jnp.broadcast_to(ko[:, d:d + 1], (8, LANE)) for d in range(DH)]
        kbc_ref[i] = jnp.concatenate(cols, axis=0).reshape(DH, 8, LANE)

    def pv_dot(h, c, p):
        return jnp.dot(vt_ref[h, :, pl.ds(c * CK, CK)], p, precision=jax.lax.Precision.DEFAULT,
                       preferred_element_type=f32)

    def ffn_dot(fb, st, ph, rp, th, sub, fr=FR):
        hcols = slice(th * 512, (th + 1) * 512)
        if ph == 0:
            xt = pltpu.bitcast(xp_ref[fb, rp * fr // 2:(rp + 1) * fr // 2, sub * LANE:(sub + 1) * LANE], bf16)
            w = pltpu.bitcast(w1p_ref[sub * 64:(sub + 1) * 64, hcols], bf16)
            o = jnp.dot(xt, w, preferred_element_type=f32)
            st["a"] = o + (bf_ref[0:1, hcols] if sub == 0 else st["a"])
            if sub == NKT - 1:
                hid = jnp.maximum(st["a"], 0.0)
                st[rp, th] = (hid * hid).astype(bf16)
        else:
            r0 = fb * FB + rp * fr
            if not isinstance(r0, int):
                r0 = pl.multiple_of(r0, fr)
            w = pltpu.bitcast(w2p_ref[th * 256:(th + 1) * 256, sub * LANE:(sub + 1) * LANE], bf16)
            o = jnp.dot(st[rp, th], w, preferred_element_type=f32)
            dst = (pl.ds(r0, fr), pl.ds(sub * LANE, LANE))
            bb_ref[dst] = o if th == 0 else o + bb_ref[dst]

    def block(h, hn, ms):
        mnxt = []
        fst = {}
        if h is not None:
            hn2 = jnp.minimum(hn + 1, H - 1)

        def vpu_piece(g, c, r, j):
            i = c * RV + r
            if j % 2 == 0:
                def terms(d):
                    kb = kbc_ref[i, d]
                    return [kb * qt_ref[hn, pl.ds(d, 1), pl.ds(g * TQ + (j + e) * LANE, LANE)] for e in range(2)]
                fst["pair"] = jax.lax.fori_loop(
                    1, DH, lambda d, a: tuple(x + t for x, t in zip(a, terms(d))), tuple(terms(0)), unroll=True)
            acc = fst["pair"][j % 2]
            s_ref[g, pl.ds((c * G8 + r) * 8, 8), pl.ds(j * LANE, LANE)] = acc
            if g == LAST_USE[c] and j == NJ - 1:
                make_kbc(hn2, i)
            return acc

        acc = None
        for u in range(NU):
            g, c = divmod(u, NC)
            if h is not None:
                s = s_ref[g, pl.ds(c * CK, CK), :].reshape(G8, 8, TQ)
                p = jnp.exp2(s - ms[g][None]).reshape(CK, TQ)
            if c == 0:
                cm = [None] * NJ
                queue = []
                rv = RVG[g] if h is not None else [0] * NC
            queue += [(g, c, r, j) for r in range(rv[c]) for j in range(NJ)]
            n = min(NPIECE[g][c], len(queue))
            mine, queue = queue[:n], queue[n:]
            L = G8 - rv[c]
            kk = pltpu.bitcast(kb_ref[hn, pl.ds((c * G8 + rv[c]) * 4, L * 4), :], bf16)[:, 0:KD]
            qq = pltpu.bitcast(qm_ref[hn, :, pl.ds(g * TQ, TQ)], bf16)
            sn = jnp.dot(kk, qq, preferred_element_type=f32)
            s_ref[g, pl.ds((c * G8 + rv[c]) * 8, L * 8), :] = sn
            pos = [max(1, int(round((k + 1) / n * (L + POFF) - POFF))) for k in range(n)] + [L]
            done = 0
            for k in range(n + 1):
                if pos[k] > done:
                    lj = colmax8(sn[done * 8:pos[k] * 8, :])
                    for j in range(NJ):
                        x = lj[:, j * LANE:(j + 1) * LANE]
                        cm[j] = x if cm[j] is None else jnp.maximum(cm[j], x)
                    done = pos[k]
                if k < n:
                    j = mine[k][3]
                    cm[j] = jnp.maximum(cm[j], vpu_piece(*mine[k]))
            if c == NC - 1:
                assert not queue
                m = jnp.concatenate(cm, axis=1)
                mnxt.append(jnp.broadcast_to(jnp.max(m, axis=0, keepdims=True), (8, TQ)))
            if h is not None:
                pv = pv_dot(h, c, p)
                acc = pv if c == 0 else pv + acc
                if c == NC - 1:
                    for j in range(NJ):
                        ot_ref[g * NJ + j, _ds(h, VROWS), :] = acc[:, j * LANE:(j + 1) * LANE]
                if u in FMAP:
                    ffn_dot(h, fst, *FMAP[u])
            elif u % 2 == 0:
                make_kbc(hn + 1, u // 2, sn[0:8, 0:LANE])
        return tuple(mnxt)

    for cp in [gw_copy, w_copy(2), xa_copy, xb_copy, w_copy(1), w_copy(0), x_copy(2), x_copy(3)] + late + [b2_copy]:
        cp.start()
    z_ref[0] = 0
    ot_ref[:, H * VROWS - 8:H * VROWS, :] = jnp.ones((S // LANE, 8, LANE), f32)

    lane = jax.lax.broadcasted_iota(jnp.int32, (RC // 2, LANE), 1)

    def head_rows(t, h, ones_row):
        vrow = jax.lax.broadcasted_iota(jnp.int32, (8, t.shape[1]), 0)
        lo = DH * h + 16
        if lo + 8 <= D:
            tail = t[lo:lo + 8, :]
        else:
            tail = jnp.concatenate([t[lo:lo + 4, :], t[lo:lo + 4, :]], axis=0)
        fill = jnp.where(vrow == 4, 1.0, 0.0) if ones_row else 0.0
        return t[DH * h:DH * h + 16, :], jnp.where(vrow < 4, tail, fill)

    def run_linked(jobs, res):
        nt = res.shape[1] // LANE
        for k, job in enumerate(jobs):
            t = k * (nt - 1) * res.shape[0] // len(jobs)
            ct, row = t // res.shape[0], t % res.shape[0] // 8 * 8
            job(res[row:row + 8, ct * LANE:(ct + 1) * LANE])

    def gate_jobs(r):
        def job(i, link):
            rows = _ds(r * (RC // GR) + i, GR)
            xb = x_ref[rows, :]
            xp_ref[r * (RC // FB) + i * GR // FB, pl.ds(i * GR % FB // 2, GR // 2), :] = after(
                pltpu.bitcast(xb, u32), link)
            gw = after(bf_ref[8:16, D:2 * D], link)
            xt = xb.astype(f32).reshape(GR // 8, 8, D)
            gl = jnp.sum((xt * gw[None]).reshape(GR, D), axis=-1, keepdims=True)
            gb_ref[rows, :] = jnp.broadcast_to(jax.nn.sigmoid(gl), (GR, LANE))
        return [lambda link, i=i: job(i, link) for i in range(RC // GR)]

    def k_proj(r, jobs=()):
        k = jnp.dot(x_ref[_ds(r, RC), :], wqkv_ref[1], preferred_element_type=f32)
        run_linked(jobs, k)
        kp = pltpu.bitcast(k.astype(bf16), u32)
        cpr = RC // CK
        for h in range(H):
            b, t0 = divmod(DH * h, LANE)
            src = kp[:, b * LANE:(b + 1) * LANE]
            if t0 + DH > LANE:
                src = jnp.where(lane >= t0, src, kp[:, (b + 1) * LANE:(b + 2) * LANE])
            if t0:
                src = pltpu.roll(src, LANE - t0, 1)
            kb_ref[h, _ds(r, RC // 2), :] = src
            for cc in range(cpr):
                kf = pltpu.bitcast(src[cc * CK // 2:cc * CK // 2 + RV * 4, :], bf16).astype(f32)
                ko_ref[h, _ds(r * cpr + cc, RV * 8), :] = kf

    def q_proj(r, jobs):
        cols = _ds(r, RC)
        qt = jax.lax.dot_general(wqkv_ref[0], x_ref[cols, :], (((0,), (1,)), ((), ())),
                                 preferred_element_type=f32)
        run_linked(jobs, qt)
        qt = (qt * QSCALE).astype(bf16).astype(f32)
        zero8 = jnp.zeros((8, RC), f32)
        for h in range(H):
            top, tail = head_rows(qt, h, False)
            qt_ref[h, 0:16, cols] = top
            qt_ref[h, 16:24, cols] = tail
            q32 = jnp.concatenate([top, tail, zero8], axis=0).astype(bf16)
            qm_ref[h, :, cols] = pltpu.bitcast(q32, u32)

    def v_proj(cols, split=1):
        xc = x_ref[cols, :]
        n = D // 2 // split
        vt = jnp.concatenate([
            jax.lax.dot_general(pltpu.bitcast(wvt_ref[i * n:(i + 1) * n, :], bf16), xc, (((1,), (1,)), ((), ())),
                                preferred_element_type=f32) for i in range(split)], axis=0)
        for h in range(H):
            top, tail = head_rows(vt, h, True)
            vt_ref[h, 0:16, cols] = top
            vt_ref[h, 16:24, cols] = tail

    gw_copy.wait()
    bf_ref[8:16, D:2 * D] = jnp.broadcast_to(gw_ref[...].astype(f32)[None, :], (8, D))
    w_copy(2).wait()
    wvt_ref[...] = pltpu.bitcast(wqkv_ref[2].T, u32)
    xa_copy.wait()
    v_proj(pl.ds(0, X0), 2)
    xb_copy.wait()
    v_proj(pl.ds(X0, RC - X0), 2)
    v_proj(_ds(1, RC))
    w_copy(1).wait()
    w_copy(0).wait()

    def proj(r, _):
        x_copy(r + 2).wait()
        k_proj(r, gate_jobs(r))
        v_proj(_ds(r + 2, RC))
        q_proj(r, gate_jobs(r + 2))
        return 0
    jax.lax.fori_loop(0, 2, proj, 0)
    for cp in late:
        cp.wait()
    bf_ref[0:8, :] = jnp.broadcast_to(b1_ref[...].astype(f32)[None, :], (8, F))

    def pack_job(src, dst, i, n, link):
        dst[pl.ds(i * n * 8, n * 8), :] = after(pltpu.bitcast(src[pl.ds(i * n * 16, n * 16), :], u32), link)
    packs = ([(w1_ref, w1p_ref, i, 1) for i in range(D // 16)]
             + [(w2_ref, w2p_ref, i, 3) for i in range(F // 48)]
             + [(wo_ref, wop_ref, i, 2) for i in range(D // 32)])
    pjobs = [lambda link, p=p: pack_job(*p, link) for p in packs]
    k_proj(2)
    k_proj(3)
    q_proj(2, pjobs[:len(pjobs) // 2])
    q_proj(3, pjobs[len(pjobs) // 2:])

    ms = block(None, 0, None)
    ms = jax.lax.fori_loop(0, H - 1, lambda h, ms: block(h, h + 1, ms), ms)
    b2_copy.wait()
    for g in range(NG):
        m_ref[g] = ms[g]
    bf_ref[8:16, 0:D] = jnp.broadcast_to(b2_ref[...].astype(f32)[None, :], (8, D))

    K1 = (NKT - 1) * LANE

    def stage(g, first=False, last=False):
        base = g if first else g - 1
        n = 1 if (first or last) else 2
        cur = 0 if first else 1
        otv = ot_ref.at[pl.ds(base * NJ, n * NJ)]
        invv = inv_ref.at[pl.ds(base * NJ, n * NJ)]
        opv = op_ref.at[pl.ds(base * NJ, n * NJ)]
        bbv = bb_ref.at[_ds(base, TQ)]
        gbv = gb_ref.at[_ds(base, TQ)]
        ov = o_ref.at[_ds(base, TQ)]

        def prep(t, k0, k1):
            h0, h1 = k0 * LANE // DH, -(-k1 * LANE // DH)
            o = jnp.concatenate([otv[t, pl.ds(h * VROWS, DH), :] * invv[t, pl.ds(h, 1), :] for h in range(h0, h1)],
                                axis=0)[k0 * LANE - h0 * DH:k1 * LANE - h0 * DH, :]
            opv[t, :, k0 * LANE:k1 * LANE] = pltpu.bitcast(o.T.astype(bf16), u32)

        def prep_early(j, link):
            t = cur * NJ + j
            sub = jax.lax.broadcasted_iota(jnp.int32, (8, LANE), 0)
            for h8 in range(0, H, 8):
                den = link
                for i in range(8):
                    den = jnp.where(sub == i, otv[t, pl.ds((h8 + i) * VROWS + DH, 1), :], den)
                invv[t, h8:h8 + 8, :] = 1.0 / den
            prep(t, 0, NKT - 1)

        def prep_late():
            for t in range(NJ):
                invv[t, H - 1:H, :] = 1.0 / otv[t, pl.ds((H - 1) * VROWS + DH, 1), :]
                prep(t, NKT - 1, NKT)

        def a1(rt, ct):
            rows = pl.ds(rt * LANE, LANE)
            cols = pl.ds(ct * LANE, LANE)
            o = pltpu.bitcast(opv[rt, :, 0:K1], bf16)
            w = pltpu.bitcast(wop_ref[0:K1 // 2, cols], bf16)
            a = jnp.dot(o, w, preferred_element_type=f32)
            gt = gbv[rows, :]
            bbv[rows, cols] = gt * a + (1.0 - gt) * (bbv[rows, cols] + bf_ref[8:9, cols])

        def a2(ct, t0, t1):
            rows = pl.ds(t0 * LANE, (t1 - t0) * LANE)
            cols = pl.ds(ct * LANE, LANE)
            o = pltpu.bitcast(opv[t0:t1, :, K1:D].reshape((t1 - t0) * LANE // 2, LANE), bf16)
            w = pltpu.bitcast(wop_ref[K1 // 2:D // 2, cols], bf16)
            a = jnp.dot(o, w, preferred_element_type=f32)
            ov[rows, cols] = (bbv[rows, cols] + gbv[rows, :] * a).astype(bf16)

        if last:
            prep_late()
            per = NJ // NLAST
            for i in range(NLAST):
                lag = 2 if i == 0 else 1
                for ct in range(NKT + lag):
                    if ct < NKT:
                        for rt in range(i * per, (i + 1) * per):
                            a1(rt, ct)
                    if ct >= lag:
                        a2(ct - lag, i * per, (i + 1) * per)
                last_copy(i).start()
            return

        if first:
            fst = {}
            jobs = [lambda fd=fd: ffn_dot(H - 1, fst, *fd, fr=FB) for fd in FDOTS if fd[1] == 0]
        else:
            jobs = [prep_late]
            for ct in range(NKT):
                jobs += [lambda rt=rt, ct=ct: a1(rt, ct) for rt in range(NJ)]
                if ct > 0:
                    jobs.append(lambda ct=ct: a2(ct - 1, 0, NJ))
            jobs.append(lambda: a2(NKT - 1, 0, NJ))
        slot = [k * (NC + 4 if first else NC) // len(jobs) for k in range(len(jobs))]
        m = m_ref[g]
        acc = None
        for c in range(NC):
            for k, job in enumerate(jobs):
                if slot[k] == c:
                    job()
            if c in PREPC:
                prep_early(PREPC.index(c), acc[0:8, 0:LANE])
            s = s_ref[g, pl.ds(c * CK, CK), :].reshape(G8, 8, TQ)
            p = jnp.exp2(s - m[None]).reshape(CK, TQ)
            pv = pv_dot(H - 1, c, p)
            acc = pv if c == 0 else pv + acc
        for j in range(NJ):
            otv[cur * NJ + j, _ds(H - 1, VROWS), :] = acc[:, j * LANE:(j + 1) * LANE]
        for k, job in enumerate(jobs):
            if slot[k] >= NC:
                job()
        if not first:
            o_copy(g - 1).start()

    stage(0, first=True)

    def tail(g, _):
        stage(g)
        return 0
    jax.lax.fori_loop(1, NG, tail, 0)
    stage(NG, last=True)
    for g in range(NG - 1):
        o_copy(g).wait()
    for i in range(NLAST):
        last_copy(i).wait()


_SCRATCH = [
    pltpu.VMEM((NG, S, TQ), f32),
    pltpu.VMEM((NC * RV, DH, 8, LANE), f32),
    pltpu.VMEM((H, VROWS, S), f32),
    pltpu.VMEM((D // 2, F), u32),
    pltpu.VMEM((F // 2, D), u32),
    pltpu.VMEM((16, F), f32),
    pltpu.VMEM((H, S // 2, LANE), u32),
    pltpu.VMEM((H, KD // 2, S), u32),
    pltpu.VMEM((H, VROWS, S), f32),
    pltpu.VMEM((S, D), f32),
    pltpu.VMEM((H, FB // 2, D), u32),
    pltpu.VMEM((S, D), bf16),
    pltpu.VMEM((H, NC * RV * 8, LANE), f32),
    pltpu.VMEM((S // LANE, H * VROWS, LANE), f32),
    pltpu.VMEM((NG, 8, TQ), f32),
    pltpu.VMEM((S, LANE), f32),
    pltpu.VMEM((D // 2, D), u32),
    pltpu.VMEM((D // 2, D), u32),
    pltpu.VMEM((S // LANE, LANE // 2, D), u32),
    pltpu.VMEM((S // LANE, H, LANE), f32),
    pltpu.VMEM((S, D), bf16),
    pltpu.VMEM((3, D, D), bf16),
    pltpu.VMEM((D, D), bf16),
    pltpu.VMEM((D, F), bf16),
    pltpu.VMEM((F, D), bf16),
    pltpu.SemaphoreType.DMA((10,)),
    pltpu.SMEM((1,), jnp.int32),
    pltpu.VMEM((F,), bf16),
    pltpu.VMEM((D,), bf16),
    pltpu.VMEM((D,), bf16),
]


@jax.jit
def pallas_gated_mix__softmax_full_mha__dense_activation_squared_relu__prompt_kernel(
    A_x: jax.Array,
    A_wqkv: jax.Array,
    A_wo: jax.Array,
    B_x: jax.Array,
    B_w1: jax.Array,
    B_b1: jax.Array,
    B_w2: jax.Array,
    B_b2: jax.Array,
    gate_w: jax.Array,
):
    del B_x
    hbm = pl.BlockSpec(memory_space=pl.ANY)
    out = pl.pallas_call(
        _kernel,
        in_specs=[hbm] * 8,
        out_specs=hbm,
        out_shape=jax.ShapeDtypeStruct((S, D), bf16),
        scratch_shapes=_SCRATCH,
        compiler_params=pltpu.CompilerParams(vmem_limit_bytes=110 * 1024 * 1024),
    )(A_x.reshape(S, D), A_wqkv, A_wo, B_w1, B_b1, B_w2, B_b2, gate_w)
    return out.reshape(1, S, D)
```

```python
import math

import jax
import jax.numpy as jnp
import jax.experimental.pallas as pl
import jax.experimental.pallas.tpu as pltpu

S = 2048
D = 640
H = 32
DH = 20
F = 1536
LANE = 128
VROWS = 24
KD = 32
NKT = D // LANE
TQ = 512
NG = S // TQ
NJ = TQ // LANE
CK = 128
NC = S // CK
G8 = CK // 8
NU = NG * NC
RC = 512
X0 = 256
FB = S // H
FR = 32
GR = 32
NLAST = 4
RV = 2
RVG = [[RV] * NC] * (NG - 1) + [[RV] * (NC - 1) + [0]]
NPIECE = [[RV * NJ] * NC] * (NG - 1) + [[8, 8, 8, 8, 8, 8, 8, 8, 8, 8, 8, 6, 8, 6, 6, 6]]
LAST_USE = {c: max(g for g in range(NG) if RVG[g][c]) for c in range(NC)}
RV0 = 4
NS0 = NC // 2 * RV0
POFF = 3
PREPC = (1, 3, 5, 7)
QSCALE = (DH ** -0.5) * math.log2(math.e)
FDOTS = [(ph, rp, th, sub) for ph in range(2) for rp in range(FB // FR) for th in range(3) for sub in range(NKT)]
FMAP = dict(zip([u for u in range(NU) if u % NC != NC - 1], FDOTS))

f32 = jnp.float32
bf16 = jnp.bfloat16
u32 = jnp.uint32


def _ds(i, n):
    return pl.ds(i * n, n) if isinstance(i, int) else pl.ds(pl.multiple_of(i * n, n), n)


def _lane_bcast(k8):
    cols = [jnp.broadcast_to(k8[:, d:d + 1], (8, LANE)) for d in range(DH)]
    return jnp.concatenate(cols, axis=0).reshape(DH, 8, LANE)


def _kernel(x_hbm, wqkv_hbm, wo_hbm, w1_hbm, b1_hbm, w2_hbm, b2_hbm, gw_hbm, o_hbm,
            s_ref, kbc_ref, qt_ref, w1p_ref, w2p_ref, bf_ref, kb_ref, qm_ref, vt_ref, bb_ref, xp_ref, x_ref,
            ko_ref, ot_ref, m_ref, gb_ref, wop_ref, wqt_ref, op_ref, inv_ref, o_ref, kbc0_ref,
            wqkv_ref, wo_ref, w1_ref, w2_ref, sems, z_ref, b1_ref, b2_ref, gw_ref):

    def x_copy(r):
        return pltpu.make_async_copy(x_hbm.at[_ds(r, RC), :], x_ref.at[_ds(r, RC), :], sems.at[r])

    def w_copy(p):
        return pltpu.make_async_copy(wqkv_hbm.at[:, pl.ds(p * D, D)], wqkv_ref.at[p], sems.at[4 + (p + 1) // 2])

    xa_copy = pltpu.make_async_copy(x_hbm.at[0:X0, :], x_ref.at[0:X0, :], sems.at[0])
    xb_copy = pltpu.make_async_copy(x_hbm.at[X0:2 * RC, :], x_ref.at[X0:2 * RC, :], sems.at[1])
    gw_copy = pltpu.make_async_copy(gw_hbm, gw_ref, sems.at[6])
    b2_copy = pltpu.make_async_copy(b2_hbm, b2_ref, sems.at[7])
    late = [pltpu.make_async_copy(w1_hbm, w1_ref, sems.at[8]),
            pltpu.make_async_copy(w2_hbm, w2_ref, sems.at[8]),
            pltpu.make_async_copy(wo_hbm, wo_ref, sems.at[8]),
            pltpu.make_async_copy(b1_hbm, b1_ref, sems.at[8])]

    def o_copy(g):
        return pltpu.make_async_copy(o_ref.at[_ds(g, TQ), :], o_hbm.at[_ds(g, TQ), :], sems.at[9])

    def last_copy(i):
        rows = pl.ds((NG - 1) * TQ + i * (TQ // NLAST), TQ // NLAST)
        return pltpu.make_async_copy(o_ref.at[rows, :], o_hbm.at[rows, :], sems.at[9])

    def colmax8(s):
        return jnp.max(s.reshape(s.shape[0] // 8, 8, s.shape[1]), axis=0) if s.shape[0] > 8 else s

    def colmax(cm):
        return jnp.broadcast_to(jnp.max(jnp.concatenate(cm, axis=1), axis=0, keepdims=True), (8, TQ))

    def after(x, link):
        lk = link if x.dtype == f32 else pltpu.bitcast(link, x.dtype)
        lk = jnp.concatenate([lk] * (x.shape[1] // LANE), axis=1)
        lk = jnp.concatenate([lk] * (x.shape[0] // 8), axis=0)
        return jnp.where(jnp.full(x.shape, z_ref[0]) != 0, lk, x)

    def make_kbc(h, i, link=None):
        ko = ko_ref[h, pl.ds(i * 8, 8), :]
        kbc_ref[i] = _lane_bcast(ko if link is None else after(ko, link))

    def score_pair(kref, h, i, col, link=None):
        def terms(d):
            kb = kref[i, d]
            return [kb * qt_ref[h, pl.ds(d, 1), pl.ds(col + e * LANE, LANE)] for e in range(2)]
        first = terms(0)
        if link is not None:
            first = [after(t, link) for t in first]
        return jax.lax.fori_loop(
            1, DH, lambda d, a: tuple(x + t for x, t in zip(a, terms(d))), tuple(first), unroll=True)

    def pv_dot(h, c, p):
        return jnp.dot(vt_ref[h, :, pl.ds(c * CK, CK)], p, precision=jax.lax.Precision.DEFAULT,
                       preferred_element_type=f32)

    def ffn_dot(fb, st, ph, rp, th, sub, fr=FR):
        hcols = slice(th * 512, (th + 1) * 512)
        if ph == 0:
            xt = pltpu.bitcast(xp_ref[fb, rp * fr // 2:(rp + 1) * fr // 2, sub * LANE:(sub + 1) * LANE], bf16)
            w = pltpu.bitcast(w1p_ref[sub * 64:(sub + 1) * 64, hcols], bf16)
            o = jnp.dot(xt, w, preferred_element_type=f32)
            st["a"] = o + (bf_ref[0:1, hcols] if sub == 0 else st["a"])
            if sub == NKT - 1:
                hid = jnp.maximum(st["a"], 0.0)
                st[rp, th] = (hid * hid).astype(bf16)
        else:
            r0 = fb * FB + rp * fr
            if not isinstance(r0, int):
                r0 = pl.multiple_of(r0, fr)
            w = pltpu.bitcast(w2p_ref[th * 256:(th + 1) * 256, sub * LANE:(sub + 1) * LANE], bf16)
            o = jnp.dot(st[rp, th], w, preferred_element_type=f32)
            dst = (pl.ds(r0, fr), pl.ds(sub * LANE, LANE))
            bb_ref[dst] = o if th == 0 else o + bb_ref[dst]

    def block(h, ms):
        first = h is None
        hn = 0 if first else h + 1
        hn2 = None if first else jnp.minimum(hn + 1, H - 1)
        cms = []
        fst = {}

        def vpu_piece(g, c, r, j, link):
            if j % 2 == 0:
                if first:
                    fst["pair"] = score_pair(kbc0_ref, 0, c * RV0 + r, g * TQ + j * LANE, link)
                else:
                    fst["pair"] = score_pair(kbc_ref, hn, c * RV + r, g * TQ + j * LANE)
            acc = fst["pair"][j % 2]
            s_ref[g, pl.ds((c * G8 + r) * 8, 8), pl.ds(j * LANE, LANE)] = acc
            if not first and g == LAST_USE[c] and j == NJ - 1:
                make_kbc(hn2, c * RV + r)
            return acc

        acc = None
        prev = None
        for u in range(NU):
            g, c = divmod(u, NC)
            if not first:
                s = s_ref[g, pl.ds(c * CK, CK), :].reshape(G8, 8, TQ)
                p = jnp.exp2(s - ms[g][None]).reshape(CK, TQ)
            if c == 0:
                cm = [None] * NJ
                queue = []
                rv = [RV0] * (NC // 2) + [0] * (NC // 2) if first else RVG[g]
            if first:
                queue += [(g,) + divmod(NS0 - NC + c, RV0) + (j,) for j in range(NJ)]
            else:
                queue += [(g, c, r, j) for r in range(rv[c]) for j in range(NJ)]
            n = len(queue) if first else min(NPIECE[g][c], len(queue))
            mine, queue = queue[:n], queue[n:]
            L = G8 - rv[c]
            kk = pltpu.bitcast(kb_ref[hn, pl.ds((c * G8 + rv[c]) * 4, L * 4), :], bf16)[:, 0:KD]
            qq = pltpu.bitcast(qm_ref[hn, :, pl.ds(g * TQ, TQ)], bf16)
            sn = jnp.dot(kk, qq, preferred_element_type=f32)
            s_ref[g, pl.ds((c * G8 + rv[c]) * 8, L * 8), :] = sn
            poff = 0 if first else POFF
            pos = [max(1, int(round((k + 1) / n * (L + poff) - poff))) for k in range(n)] + [L]
            done = 0
            for k in range(n + 1):
                if pos[k] > done:
                    lj = colmax8(sn[done * 8:pos[k] * 8, :])
                    for j in range(NJ):
                        x = lj[:, j * LANE:(j + 1) * LANE]
                        cm[j] = x if cm[j] is None else jnp.maximum(cm[j], x)
                    done = pos[k]
                if k < n:
                    link = None
                    if first and k % 2 == 0:
                        q = pos[k] - 6
                        src = sn if (q >= 0 or prev is None) else prev
                        q = max(q, 0) if src is sn else q + prev.shape[0] // 8
                        link = src[q * 8:(q + 1) * 8, 0:LANE]
                    j = mine[k][3]
                    cm[j] = jnp.maximum(cm[j], vpu_piece(*mine[k], link))
            prev = sn
            if c == NC - 1:
                assert not queue
                cms.append(cm if first else colmax(cm))
            if not first:
                pv = pv_dot(h, c, p)
                acc = pv if c == 0 else pv + acc
                if c == NC - 1:
                    for j in range(NJ):
                        ot_ref[g * NJ + j, _ds(h, VROWS), :] = acc[:, j * LANE:(j + 1) * LANE]
                if u in FMAP:
                    ffn_dot(h, fst, *FMAP[u])
            elif u % 2 == 0:
                make_kbc(1, u // 2, sn[0:8, 0:LANE])
        if first:
            cms = [colmax([jnp.maximum(cms[g][j], ms[g, j]) for j in range(NJ)]) for g in range(NG)]
        return tuple(cms)

    for cp in [gw_copy, w_copy(0), xa_copy, xb_copy, w_copy(1), w_copy(2), x_copy(2), x_copy(3)] + late + [b2_copy]:
        cp.start()
    z_ref[0] = 0
    ot_ref[:, H * VROWS - 8:H * VROWS, :] = jnp.ones((S // LANE, 8, LANE), f32)

    lane = jax.lax.broadcasted_iota(jnp.int32, (RC // 2, LANE), 1)

    def head_rows(t, h, ones_row):
        vrow = jax.lax.broadcasted_iota(jnp.int32, (8, t.shape[1]), 0)
        lo = DH * h + 16
        if lo + 8 <= D:
            tail = t[lo:lo + 8, :]
        else:
            tail = jnp.concatenate([t[lo:lo + 4, :], t[lo:lo + 4, :]], axis=0)
        fill = jnp.where(vrow == 4, 1.0, 0.0) if ones_row else 0.0
        return t[DH * h:DH * h + 16, :], jnp.where(vrow < 4, tail, fill)

    def run_linked(jobs, res, skip):
        nt = res.shape[1] // LANE - skip
        for k, job in enumerate(jobs):
            t = k * nt * res.shape[0] // len(jobs)
            ct, row = t // res.shape[0], t % res.shape[0] // 8 * 8
            job(res[row:row + 8, ct * LANE:(ct + 1) * LANE])

    def gate_jobs(r):
        def job(i, link):
            rows = _ds(r * (RC // GR) + i, GR)
            xb = x_ref[rows, :]
            xp_ref[r * (RC // FB) + i * GR // FB, pl.ds(i * GR % FB // 2, GR // 2), :] = after(
                pltpu.bitcast(xb, u32), link)
            gw = after(bf_ref[8:16, D:2 * D], link)
            xt = xb.astype(f32).reshape(GR // 8, 8, D)
            gl = jnp.sum((xt * gw[None]).reshape(GR, D), axis=-1, keepdims=True)
            gb_ref[rows, :] = jnp.broadcast_to(jax.nn.sigmoid(gl), (GR, LANE))
        return [lambda link, i=i: job(i, link) for i in range(RC // GR)]

    def k_proj(r, jobs, early):
        k = jnp.dot(x_ref[_ds(r, RC), :], wqkv_ref[1], preferred_element_type=f32)
        run_linked(jobs, k, 1 if early else 0)
        kp = pltpu.bitcast(k.astype(bf16), u32)
        cpr = RC // CK
        for h in range(H):
            b, t0 = divmod(DH * h, LANE)
            src = kp[:, b * LANE:(b + 1) * LANE]
            if t0 + DH > LANE:
                src = jnp.where(lane >= t0, src, kp[:, (b + 1) * LANE:(b + 2) * LANE])
            if t0:
                src = pltpu.roll(src, LANE - t0, 1)
            kb_ref[h, _ds(r, RC // 2), :] = src
            for cc in range(cpr):
                kf = pltpu.bitcast(src[cc * CK // 2:cc * CK // 2 + RV * 4, :], bf16).astype(f32)
                ko_ref[h, _ds(r * cpr + cc, RV * 8), :] = kf
        if early:
            k0 = k[:, 0:LANE].astype(bf16).astype(f32)
            for cc in range(cpr):
                for i in range(RV0):
                    kbc0_ref[r * (cpr * RV0) + cc * RV0 + i] = _lane_bcast(k0[cc * CK + i * 8:cc * CK + (i + 1) * 8, :])

    def q_proj(cols, split=1, jobs=()):
        xc = x_ref[cols, :]
        n = D // 2 // split
        qt = jnp.concatenate([
            jax.lax.dot_general(pltpu.bitcast(wqt_ref[i * n:(i + 1) * n, :], bf16), xc, (((1,), (1,)), ((), ())),
                                preferred_element_type=f32) for i in range(split)], axis=0)
        run_linked(jobs, qt, 1)
        qt = (qt * QSCALE).astype(bf16).astype(f32)
        zero8 = jnp.zeros((8, qt.shape[1]), f32)
        for h in range(H):
            top, tail = head_rows(qt, h, False)
            qt_ref[h, 0:16, cols] = top
            qt_ref[h, 16:24, cols] = tail
            q32 = jnp.concatenate([top, tail, zero8], axis=0).astype(bf16)
            qm_ref[h, :, cols] = pltpu.bitcast(q32, u32)

    def v_proj(r, jobs=()):
        cols = _ds(r, RC)
        vt = jax.lax.dot_general(wqkv_ref[2], x_ref[cols, :], (((0,), (1,)), ((), ())),
                                 preferred_element_type=f32)
        run_linked(jobs, vt, 0)
        for h in range(H):
            top, tail = head_rows(vt, h, True)
            vt_ref[h, 0:16, cols] = top
            vt_ref[h, 16:24, cols] = tail

    gw_copy.wait()
    bf_ref[8:16, D:2 * D] = jnp.broadcast_to(gw_ref[...].astype(f32)[None, :], (8, D))
    w_copy(0).wait()
    wqt_ref[...] = pltpu.bitcast(wqkv_ref[0].T, u32)
    xa_copy.wait()
    q_proj(pl.ds(0, X0), 2)
    xb_copy.wait()
    q_proj(pl.ds(X0, RC - X0), 2)
    q_proj(_ds(1, RC))
    w_copy(1).wait()
    w_copy(2).wait()

    def proj(r, _):
        x_copy(r + 2).wait()
        k_proj(r, gate_jobs(r), True)
        v_proj(r)
        q_proj(_ds(r + 2, RC), jobs=gate_jobs(r + 2))
        return 0
    jax.lax.fori_loop(0, 2, proj, 0)
    for cp in late:
        cp.wait()
    bf_ref[0:8, :] = jnp.broadcast_to(b1_ref[...].astype(f32)[None, :], (8, F))

    def pack_job(src, dst, i, n, link):
        dst[pl.ds(i * n * 8, n * 8), :] = after(pltpu.bitcast(src[pl.ds(i * n * 16, n * 16), :], u32), link)
    packs = ([(w1_ref, w1p_ref, i, 1) for i in range(D // 16)]
             + [(w2_ref, w2p_ref, i, 3) for i in range(F // 48)]
             + [(wo_ref, wop_ref, i, 2) for i in range(D // 32)])
    pjobs = [lambda link, p=p: pack_job(*p, link) for p in packs]

    m0 = {}

    def head0_job(g, i, j, link):
        c, r = divmod(i, RV0)
        for e, v in enumerate(score_pair(kbc0_ref, 0, i, g * TQ + j * LANE, link)):
            s_ref[g, pl.ds((c * G8 + r) * 8, 8), pl.ds((j + e) * LANE, LANE)] = v
            m0[g, j + e] = jnp.maximum(m0[g, j + e], v) if (g, j + e) in m0 else v
    hjobs = [lambda link, a=(g, i, j): head0_job(*a, link)
             for g in range(NG) for i in range(NS0 - NC) for j in range(0, NJ, 2)]
    cut = [int(round(w * len(hjobs) / 6)) for w in (0, 2, 4, 5, 6)]

    def mix(a, b):
        keyed = [((k + 0.5) / len(js), j) for js in (a, b) for k, j in enumerate(js)]
        return [j for _, j in sorted(keyed, key=lambda t: t[0])]
    k_proj(2, hjobs[cut[0]:cut[1]], False)
    k_proj(3, hjobs[cut[1]:cut[2]], False)
    v_proj(2, mix(pjobs[:len(pjobs) // 2], hjobs[cut[2]:cut[3]]))
    v_proj(3, mix(pjobs[len(pjobs) // 2:], hjobs[cut[3]:cut[4]]))

    ms = block(None, m0)
    ms = jax.lax.fori_loop(0, H - 1, block, ms)
    b2_copy.wait()
    for g in range(NG):
        m_ref[g] = ms[g]
    bf_ref[8:16, 0:D] = jnp.broadcast_to(b2_ref[...].astype(f32)[None, :], (8, D))

    K1 = (NKT - 1) * LANE

    def stage(g, first=False, last=False):
        base = g if first else g - 1
        n = 1 if (first or last) else 2
        cur = 0 if first else 1
        otv = ot_ref.at[pl.ds(base * NJ, n * NJ)]
        invv = inv_ref.at[pl.ds(base * NJ, n * NJ)]
        opv = op_ref.at[pl.ds(base * NJ, n * NJ)]
        bbv = bb_ref.at[_ds(base, TQ)]
        gbv = gb_ref.at[_ds(base, TQ)]
        ov = o_ref.at[_ds(base, TQ)]

        def prep(t, k0, k1):
            h0, h1 = k0 * LANE // DH, -(-k1 * LANE // DH)
            o = jnp.concatenate([otv[t, pl.ds(h * VROWS, DH), :] * invv[t, pl.ds(h, 1), :] for h in range(h0, h1)],
                                axis=0)[k0 * LANE - h0 * DH:k1 * LANE - h0 * DH, :]
            opv[t, :, k0 * LANE:k1 * LANE] = pltpu.bitcast(o.T.astype(bf16), u32)

        def prep_early(j, link):
            t = cur * NJ + j
            sub = jax.lax.broadcasted_iota(jnp.int32, (8, LANE), 0)
            for h8 in range(0, H, 8):
                den = link
                for i in range(8):
                    den = jnp.where(sub == i, otv[t, pl.ds((h8 + i) * VROWS + DH, 1), :], den)
                invv[t, h8:h8 + 8, :] = 1.0 / den
            prep(t, 0, NKT - 1)

        def prep_late():
            for t in range(NJ):
                invv[t, H - 1:H, :] = 1.0 / otv[t, pl.ds((H - 1) * VROWS + DH, 1), :]
                prep(t, NKT - 1, NKT)

        def a1(rt, ct):
            rows = pl.ds(rt * LANE, LANE)
            cols = pl.ds(ct * LANE, LANE)
            o = pltpu.bitcast(opv[rt, :, 0:K1], bf16)
            w = pltpu.bitcast(wop_ref[0:K1 // 2, cols], bf16)
            a = jnp.dot(o, w, preferred_element_type=f32)
            gt = gbv[rows, :]
            bbv[rows, cols] = gt * a + (1.0 - gt) * (bbv[rows, cols] + bf_ref[8:9, cols])

        def a2(ct, t0, t1):
            rows = pl.ds(t0 * LANE, (t1 - t0) * LANE)
            cols = pl.ds(ct * LANE, LANE)
            o = pltpu.bitcast(opv[t0:t1, :, K1:D].reshape((t1 - t0) * LANE // 2, LANE), bf16)
            w = pltpu.bitcast(wop_ref[K1 // 2:D // 2, cols], bf16)
            a = jnp.dot(o, w, preferred_element_type=f32)
            ov[rows, cols] = (bbv[rows, cols] + gbv[rows, :] * a).astype(bf16)

        if last:
            prep_late()
            per = NJ // NLAST
            for i in range(NLAST):
                lag = 2 if i == 0 else 1
                for ct in range(NKT + lag):
                    if ct < NKT:
                        for rt in range(i * per, (i + 1) * per):
                            a1(rt, ct)
                    if ct >= lag:
                        a2(ct - lag, i * per, (i + 1) * per)
                last_copy(i).start()
            return

        if first:
            fst = {}
            jobs = [lambda fd=fd: ffn_dot(H - 1, fst, *fd, fr=FB) for fd in FDOTS if fd[1] == 0]
        else:
            jobs = [prep_late]
            for ct in range(NKT):
                jobs += [lambda rt=rt, ct=ct: a1(rt, ct) for rt in range(NJ)]
                if ct > 0:
                    jobs.append(lambda ct=ct: a2(ct - 1, 0, NJ))
            jobs.append(lambda: a2(NKT - 1, 0, NJ))
        slot = [k * (NC + 4 if first else NC) // len(jobs) for k in range(len(jobs))]
        m = m_ref[g]
        acc = None
        for c in range(NC):
            for k, job in enumerate(jobs):
                if slot[k] == c:
                    job()
            if c in PREPC:
                prep_early(PREPC.index(c), acc[0:8, 0:LANE])
            s = s_ref[g, pl.ds(c * CK, CK), :].reshape(G8, 8, TQ)
            p = jnp.exp2(s - m[None]).reshape(CK, TQ)
            pv = pv_dot(H - 1, c, p)
            acc = pv if c == 0 else pv + acc
        for j in range(NJ):
            otv[cur * NJ + j, _ds(H - 1, VROWS), :] = acc[:, j * LANE:(j + 1) * LANE]
        for k, job in enumerate(jobs):
            if slot[k] >= NC:
                job()
        if not first:
            o_copy(g - 1).start()

    stage(0, first=True)

    def tail(g, _):
        stage(g)
        return 0
    jax.lax.fori_loop(1, NG, tail, 0)
    stage(NG, last=True)
    for g in range(NG - 1):
        o_copy(g).wait()
    for i in range(NLAST):
        last_copy(i).wait()


_SCRATCH = [
    pltpu.VMEM((NG, S, TQ), f32),
    pltpu.VMEM((NC * RV, DH, 8, LANE), f32),
    pltpu.VMEM((H, VROWS, S), f32),
    pltpu.VMEM((D // 2, F), u32),
    pltpu.VMEM((F // 2, D), u32),
    pltpu.VMEM((16, F), f32),
    pltpu.VMEM((H, S // 2, LANE), u32),
    pltpu.VMEM((H, KD // 2, S), u32),
    pltpu.VMEM((H, VROWS, S), f32),
    pltpu.VMEM((S, D), f32),
    pltpu.VMEM((H, FB // 2, D), u32),
    pltpu.VMEM((S, D), bf16),
    pltpu.VMEM((H, NC * RV * 8, LANE), f32),
    pltpu.VMEM((S // LANE, H * VROWS, LANE), f32),
    pltpu.VMEM((NG, 8, TQ), f32),
    pltpu.VMEM((S, LANE), f32),
    pltpu.VMEM((D // 2, D), u32),
    pltpu.VMEM((D // 2, D), u32),
    pltpu.VMEM((S // LANE, LANE // 2, D), u32),
    pltpu.VMEM((S // LANE, H, LANE), f32),
    pltpu.VMEM((S, D), bf16),
    pltpu.VMEM((NS0, DH, 8, LANE), f32),
    pltpu.VMEM((3, D, D), bf16),
    pltpu.VMEM((D, D), bf16),
    pltpu.VMEM((D, F), bf16),
    pltpu.VMEM((F, D), bf16),
    pltpu.SemaphoreType.DMA((10,)),
    pltpu.SMEM((1,), jnp.int32),
    pltpu.VMEM((F,), bf16),
    pltpu.VMEM((D,), bf16),
    pltpu.VMEM((D,), bf16),
]


@jax.jit
def pallas_gated_mix__softmax_full_mha__dense_activation_squared_relu__prompt_kernel(
    A_x: jax.Array,
    A_wqkv: jax.Array,
    A_wo: jax.Array,
    B_x: jax.Array,
    B_w1: jax.Array,
    B_b1: jax.Array,
    B_w2: jax.Array,
    B_b2: jax.Array,
    gate_w: jax.Array,
):
    del B_x
    hbm = pl.BlockSpec(memory_space=pl.ANY)
    out = pl.pallas_call(
        _kernel,
        in_specs=[hbm] * 8,
        out_specs=hbm,
        out_shape=jax.ShapeDtypeStruct((S, D), bf16),
        scratch_shapes=_SCRATCH,
        compiler_params=pltpu.CompilerParams(vmem_limit_bytes=110 * 1024 * 1024),
    )(A_x.reshape(S, D), A_wqkv, A_wo, B_w1, B_b1, B_w2, B_b2, gate_w)
    return out.reshape(1, S, D)
```
